```python
import jax
import jax.numpy as jnp

def _softmax(x, axis=-1):
    return jax.nn.softmax(x, axis=axis)
def _gelu(x):
    return jax.nn.gelu(x, approximate=True)
def _silu(x):
    return jax.nn.silu(x)
def _sigmoid(x):
    return jax.nn.sigmoid(x)
def _layernorm(x, axis=-1, eps=1e-5):
    m = jnp.mean(x, axis=axis, keepdims=True)
    v = jnp.var(x, axis=axis, keepdims=True)
    return (x - m) / jnp.sqrt(v + eps)
def _scatter_add(tgt, idx, src, axis=0):
    return tgt.at[idx].add(src)
def _segment_sum(src, seg, n):
    return jax.ops.segment_sum(src, seg, n)
class _Rng:
    def __init__(self, key):
        self._k = key
    def _next(self):
        self._k, sub = jax.random.split(self._k)
        return sub
    def normal(self, shape):
        return jax.random.normal(self._next(), shape, dtype=jnp.bfloat16)
    def randint(self, lo, hi, shape):
        return jax.random.randint(self._next(), shape, lo, hi, dtype=jnp.int32)
    def uniform(self, shape, lo=0.0, hi=1.0):
        return jax.random.uniform(self._next(), shape, jnp.bfloat16, lo, hi)
    def permutation(self, n):
        return jax.random.permutation(self._next(), n)


kernel_name = 'standalone__modern_conv_block_convnext_v2__vision'

def setup_inputs():
    _rng = _Rng(jax.random.key(int.from_bytes(__import__("os").urandom(4), "little")))
    _w = (lambda a: (lambda t: t.astype(jnp.bfloat16) if jnp.issubdtype(t.dtype, jnp.floating) else t)(jnp.asarray(a)))
    H = W = 512
    C = 96
    K = 3
    return {
        "x": _w((lambda *s: _rng.normal(s) * 0.05)(1, H, W, C)),
        "dw": _w((lambda *s: _rng.normal(s) * 0.05)(K, K, C)),
        "w1": _w((lambda *s: _rng.normal(s) * 0.05)(C, 4 * C)),
        "w2": _w((lambda *s: _rng.normal(s) * 0.05)(4 * C, C)),
        "grn_gamma": _w((lambda *s: _rng.normal(s) * 0.05)(4 * C)),
        "grn_beta": _w((lambda *s: _rng.normal(s) * 0.05)(4 * C)),
    }

def reference(x, dw, w1, w2, grn_gamma, grn_beta):
    B, H, W, C = x.shape
    K = dw.shape[0]
    pad = K // 2
    xp = jnp.pad(x, ((0,0),(pad,pad),(pad,pad),(0,0)))
    out = jnp.zeros_like(x)
    for i in range(K):
        for j in range(K):
            out = out + xp[:, i:i+H, j:j+W, :] * dw[i, j][None, None, None, :]
    h = _layernorm(out, axis=-1)
    h = jnp.einsum('bhwc,ce->bhwe', h, w1)
    h = _gelu(h)
    gx = jnp.sqrt((h * h).sum(axis=(1, 2), keepdims=True) + 1e-6)
    nx = gx / (gx.mean(axis=-1, keepdims=True) + 1e-6)
    h = grn_gamma * (h * nx) + grn_beta + h
    h = jnp.einsum('bhwe,ec->bhwc', h, w2)
    return x + h
```

```python
import math

import jax
import jax.numpy as jnp
from jax import lax
import jax.experimental.pallas as pl
import jax.experimental.pallas.tpu as pltpu

F32, BF16, U32 = jnp.float32, jnp.bfloat16, jnp.uint32
C, E, NG, NT = 96, 384, 12, 4
NP = 256
_C0 = math.sqrt(2.0 / math.pi)
_K = (_C0 * 0.044715) ** (1.0 / 3.0)
_B = _C0 / _K
_GS = 0.5 / _K
W1, S1, S2, WB = 96, 288, 360, 432


def build(U=4, MC=64, SA=5, RA=3, do1=True, do2=True, order1="cba", flags=None, dbg=False):
    NB = NP // U
    NI = NP // (SA + RA)
    NS, NR = SA * NI, RA * NI
    NM = E // MC

    def kern(x_hbm, xn_hbm, dw_ref, w1_ref, w2t_ref, gam_ref, bet_ref, o_hbm,
             G, wb, rb, w2s, bias, zs, sem):
        x32 = x_hbm.bitcast(U32)
        G16 = G.bitcast(BF16)
        zs[0] = 0
        lane = lax.broadcasted_iota(jnp.int32, (8, 128), 1)

        def in_hi(p0, n, dst, s):
            return pltpu.make_async_copy(x32.at[pl.ds(p0 - 1, n), 1], dst.at[:, :, pl.ds(0, 4)], s)

        def in_lo(p0, n, dst, s):
            return pltpu.make_async_copy(x32.at[pl.ds(p0, n), 0], dst.at[:, :, pl.ds(4, 4)], s)

        def prep_weights():
            d = dw_ref[...].astype(F32)
            rows = [d[i, j:j + 1, :] for i in range(3) for j in range(3)]
            dm = jnp.concatenate(rows + [jnp.zeros((128 - 9, C), F32)], axis=0)
            dm = jnp.concatenate([dm, jnp.zeros((128, 128 - C), F32)], axis=1)
            dt = dm.T[:C]
            r = lax.broadcasted_iota(jnp.int32, (C, 128), 0)
            k = lax.broadcasted_iota(jnp.int32, (C, 128), 1)
            diag = (r & 7) == (k & 7)
            slot = k >> 3
            outs = []
            for o in range(2):
                a = jnp.zeros((C, 128), F32)
                for i in range(3):
                    ri = i + o
                    for j in range(3):
                        s = ((ri >> 1) * 3 + j) * 2 + (ri & 1)
                        col = jnp.broadcast_to(dt[:, i * 3 + j:i * 3 + j + 1], (C, 128))
                        a = jnp.where(diag & (slot == s), col, a)
                outs.append(a)
            for g in range(NG):
                wb[0, 8 * g:8 * g + 8] = pltpu.bitcast(
                    jnp.concatenate([outs[0][8 * g:8 * g + 8], outs[1][8 * g:8 * g + 8]], axis=0).astype(BF16), U32)
            w = w1_ref[...].astype(F32)
            w = w - jnp.sum(w, axis=0, keepdims=True) * (1.0 / C)
            w = jnp.concatenate([w, jnp.zeros((128 - C, E), F32)], axis=0)
            wb[0, W1:W1 + E // 2] = pltpu.bitcast(w.T.astype(BF16), U32)

        def shift(v):
            r = [pltpu.roll(t, 1, 1) for t in v]
            l = [pltpu.roll(t, 127, 1) for t in v]
            z = jnp.zeros((8, 128), U32)
            sr = [jnp.where(lane == 0, r[j - 1] if j > 0 else z, r[j]) for j in range(NT)]
            sl = [jnp.where(lane == 127, l[j + 1] if j < NT - 1 else z, l[j]) for j in range(NT)]
            return sr, sl

        def stage_a0(g, new, sb):
            v = [new[4 * g + j] for j in range(NT)]
            sr, sl = shift(v)
            for j in range(NT):
                sb[0, 4 * g + j] = sr[j]
                sb[1, 4 * g + j] = sl[j]
            return sr, v, sl

        def stage_a(g, old, new, sb, c_out):
            o3 = [(sb[0, 4 * g + j], old[4 * g + j], sb[1, 4 * g + j]) for j in range(NT)]
            sr, v, sl = stage_a0(g, new, sb)
            cols = [jnp.concatenate([*o3[j], sr[j], v[j], sl[j]], axis=0) for j in range(NT)]
            rhs = pltpu.bitcast(jnp.concatenate(cols, axis=1), BF16)
            res = jnp.dot(pltpu.bitcast(wb[0, 8 * g:8 * g + 8], BF16)[:, :C], rhs, preferred_element_type=F32)
            for o in range(2):
                for j in range(NT):
                    c_out[4 * o + j, 8 * g:8 * g + 8, :] = res[8 * o:8 * o + 8, 128 * j:128 * j + 128]

        def tree(v):
            while len(v) > 1:
                v = [v[i] + v[i + 1] if i + 1 < len(v) else v[i] for i in range(0, len(v), 2)]
            return v[0]

        def stage_b1(q, c_in, zero):
            s1 = s2 = None
            for g in range(NG):
                c = c_in[q, 8 * g:8 * g + 8]
                s1 = c if s1 is None else s1 + c
                s2 = c * c if s2 is None else s2 + c * c
            wb[zero, S1 + 9 * q:S1 + 9 * q + 8] = pltpu.bitcast(s1, U32)
            wb[zero, S2 + 9 * q:S2 + 9 * q + 8] = pltpu.bitcast(s2, U32)

        def stage_b2():
            s1 = tree([pltpu.bitcast(wb[0, pl.ds(S1 + i, 8, stride=9), :], F32) for i in range(8)])
            s2 = tree([pltpu.bitcast(wb[0, pl.ds(S2 + i, 8, stride=9), :], F32) for i in range(8)])
            v = jnp.maximum(s2 - s1 * s1 * (1.0 / C), 0.0)
            rb[...] = lax.rsqrt(v * (1.0 / (C * _K * _K)) + 1e-5 / (_K * _K))

        def stage_b3(q, c_in, z16, zrow):
            o, j = divmod(q, NT)
            z16[pl.ds(zrow + o, 1), :, 128 * j:128 * j + 128] = (c_in[q] * rb[q:q + 1])[None].astype(BF16)

        def stage_b(q, c_in, z16, zrow, zero):
            if q < 8:
                stage_b1(q, c_in, zero)
            elif q == 8:
                stage_b2()
            else:
                for t in range(3 * (q - 9), min(3 * (q - 9) + 3, 8)):
                    stage_b3(t, c_in, z16, zrow + zero)

        def stage_c(m, rhs, g16, grow, acc):
            lhs = pltpu.bitcast(wb[0, W1 + m * MC // 2:W1 + (m + 1) * MC // 2], BF16)[:, :C]
            z = jnp.dot(lhs, rhs, preferred_element_type=F32)
            gl = z + z * jnp.tanh(z * (z * z + _B))
            g16[pl.ds(grow, 1), m * MC:(m + 1) * MC, :] = gl[None].astype(BF16)
            if acc is not None:
                sq = gl * gl
                acc[m * MC:(m + 1) * MC, :] += (sq[:, 0:128] + sq[:, 128:256]) + (sq[:, 256:384] + sq[:, 384:512])

        def pass1(xb, sb, cb0, cb1, zb, acc):
            cb = (cb0, cb1)
            z16 = zb.bitcast(BF16)

            def blk(b, slot):
                return [in_hi(b * U + 2, U + 1, xb.at[slot], sem.at[slot]),
                        in_lo(b * U + 2, U + 1, xb.at[slot], sem.at[2 + slot])]

            def last_blk(slot):
                p0 = (NB - 1) * U + 2
                r = [in_hi(p0, U - 1, xb.at[slot, pl.ds(0, U - 1)], sem.at[slot])]
                if U > 2:
                    r.append(in_lo(p0, U - 2, xb.at[slot, pl.ds(0, U - 2)], sem.at[2 + slot]))
                return r

            pa = in_hi(1, 2, xb.at[1, pl.ds(1, 2)], sem.at[1])
            pb = in_lo(0, 3, xb.at[1, pl.ds(0, 3)], sem.at[3])
            pa.start()
            pb.start()
            for c_ in blk(0, 0):
                c_.start()
            prep_weights()
            acc[...] = jnp.zeros_like(acc)
            pa.wait()
            pb.wait()
            xb[1, 0, :, 0:4, :] = jnp.zeros((48, 4, 128), U32)
            for g in range(NG):
                stage_a0(g, xb.at[1, 0], sb)
            for g in range(NG):
                stage_a(g, xb.at[1, 0], xb.at[1, 1], sb, cb[0].at[0])
            for g in range(NG):
                stage_a(g, xb.at[1, 1], xb.at[1, 2], sb, cb[1].at[0])
                stage_b(g, cb[0].at[0], z16, 0, 0)

            def body1(b, _):
                slot = b & 1
                zero = zs[0]

                @pl.when(b < NB - 1)
                def _():
                    for c_ in blk(b, slot):
                        c_.wait()

                @pl.when(b == NB - 1)
                def _():
                    for c_ in last_blk(slot):
                        c_.wait()
                    xb[slot, U - 2, :, 4:8, :] = jnp.zeros((48, 4, 128), U32)

                @pl.when(b < NB - 2)
                def _():
                    for c_ in blk(b + 1, 1 - slot):
                        c_.start()

                @pl.when(b == NB - 2)
                def _():
                    for c_ in last_blk(1 - slot):
                        c_.start()

                for u in range(U):
                    grow = 2 * jnp.maximum(b * U + u - NR, 0)
                    e = u & 1
                    nq = 2 * NM
                    for q in range(nq):
                        for st in order1:
                            if st == "c":
                                stage_c(q % NM, z16[2 * e + q // NM], G16, grow + q // NM, acc)
                            for g in range(q * NG // nq, (q + 1) * NG // nq):
                                if st == "b":
                                    stage_b(g, cb[1 - e].at[zero], z16, 2 * (1 - e), zero)
                                if st == "a":
                                    stage_a(g, xb.at[slot, u], xb.at[slot, u + 1], sb, cb[e].at[0])
                return 0

            lax.fori_loop(0, NB, body1, 0)

            ss = jnp.sum(acc[...].T, axis=0, keepdims=True)
            gx = jnp.sqrt(ss * (_GS * _GS) + 1e-6)
            nx = gx / (jnp.sum(gx, axis=1, keepdims=True) * (1.0 / E) + 1e-6)
            gam = gam_ref[...].astype(F32).reshape(1, E)
            bet = bet_ref[...].astype(F32).reshape(1, E)
            w2 = w2t_ref[...].astype(F32)
            w2s.bitcast(BF16)[...] = (w2 * ((gam * nx + 1.0) * _GS)).astype(BF16)
            bias[...] = jnp.broadcast_to(jnp.sum(w2 * bet, axis=1, keepdims=True), (C, 128))

            if dbg:
                def dd(buf):
                    buf[...] = jnp.zeros_like(buf)
                    buf[0, :, 0:384] = jnp.broadcast_to(ss, (C, E)).astype(BF16)
                    buf[1, :, 0:384] = jnp.broadcast_to(gam, (C, E)).astype(BF16)
                    buf[2, :, 0:384] = jnp.broadcast_to(bet, (C, E)).astype(BF16)
                    buf[3, :, 0:384] = w2s.bitcast(BF16)[...]
                    buf[4] = G16[0, 0:96]
                    buf[5] = z16[0]
                    buf[6, :, 0:128] = cb0[0, 0].astype(BF16)
                    buf[6, :, 128:256] = pltpu.bitcast(wb[0, 0:48], BF16)
                    buf[6, :, 256:384] = pltpu.bitcast(wb[0, W1:W1 + 48], BF16)
                    buf[6, :, 384:512] = bias[...].astype(BF16)
                    buf[7, 0:64, 0:128] = pltpu.bitcast(wb[0, S1:S1 + 64], F32).astype(BF16)
                    buf[7, 0:64, 128:256] = pltpu.bitcast(wb[0, S2:S2 + 64], F32).astype(BF16)
                    buf[7, 0:16, 256:384] = jnp.concatenate([rb[...], rb[...]], axis=0).astype(BF16)
                    buf[7, :, 384:512] = acc[0:96].astype(BF16)
                    for q in range(4):
                        buf[1, :, 128 * q:128 * q + 128] = cb0[0, q].astype(BF16)
                        buf[2, :, 128 * q:128 * q + 128] = cb1[0, q].astype(BF16)
                    buf[3] = z16[2]
                    pltpu.sync_copy(buf, o_hbm.at[pl.ds(0, 8)])
                pl.run_scoped(dd, pltpu.VMEM((8, C, 512), BF16))

        if do1:
            pl.run_scoped(
                pass1,
                pltpu.VMEM((2, U + 1, 48, 8, 128), U32),
                pltpu.VMEM((2, 48, 8, 128), U32),
                pltpu.VMEM((1, 8, C, 128), F32), pltpu.VMEM((1, 8, C, 128), F32),
                pltpu.VMEM((4, C // 2, 512), U32),
                pltpu.VMEM((E, 128), F32),
            )

        def pass2(xs, xr, orr, sb, cb, zb, gt):
            z16 = zb.bitcast(BF16)
            gt16 = gt.bitcast(BF16)

            def s_in(i, slot):
                return pltpu.make_async_copy(xn_hbm.at[pl.ds(2 * (NR + SA * i), 2 * SA)], xs.at[slot], sem.at[4 + slot])

            def s_out(i, slot):
                return pltpu.make_async_copy(xs.at[slot], o_hbm.at[pl.ds(2 * (NR + SA * i), 2 * SA)], sem.at[7 + slot])

            def r_out(i, slot):
                return pltpu.make_async_copy(orr.at[slot], o_hbm.at[pl.ds(2 * RA * i, 2 * RA)], sem.at[10 + slot])

            def r_in(i):
                r = []
                for t in range(RA):
                    p = RA * i + 1 + t
                    r.append(in_hi(p, 1, xr.at[pl.ds(p % 7, 1)], sem.at[0]))
                    r.append(in_lo(p, 1, xr.at[pl.ds(p % 7, 1)], sem.at[1]))
                return r

            p0 = in_lo(0, 1, xr.at[pl.ds(0, 1)], sem.at[2])
            p0.start()
            for c_ in r_in(0):
                c_.start()
            s_in(0, 0).start()
            p0.wait()
            xr[0, :, 0:4, :] = jnp.zeros((48, 4, 128), U32)
            for g in range(NG):
                stage_a0(g, xr.at[0], sb)

            def mm2(rhs):
                o = jnp.dot(w2s.bitcast(BF16)[...], rhs, preferred_element_type=F32)
                bb = bias[...]
                return o + jnp.concatenate([bb] * NT, axis=1)

            def body2(i, s3):
                zero = zs[0]
                s3p = jnp.where(s3 == 0, 2, s3 - 1)
                s3n = jnp.where(s3 == 2, 0, s3 + 1)
                s2 = i & 1
                for c_ in r_in(i):
                    c_.wait()
                s_in(i, s3).wait()

                @pl.when(i >= 1)
                def _():
                    s_out(i - 1, s3p).start()
                    r_out(i - 1, 1 - s2).start()

                @pl.when(i >= 2)
                def _():
                    s_out(i - 2, s3n).wait()
                    r_out(i - 2, s2).wait()

                @pl.when(i < NI - 1)
                def _():
                    for c_ in r_in(i + 1):
                        c_.start()
                    s_in(i + 1, s3n).start()

                P = [xr.at[(RA * i + t) % 7] for t in range(RA + 1)]

                def ds(r):
                    o = mm2(G16[2 * SA * i + r])
                    xs[s3, r] = (xs[s3, r].astype(F32) + o).astype(BF16)

                def dr(t, o_):
                    o = mm2(gt16[o_])
                    src, lo = (P[t], 8) if o_ == 0 else (P[t + 1], 0)
                    xx = jnp.concatenate([
                        jnp.concatenate([pltpu.bitcast(src[4 * g + j], BF16).astype(F32)[lo:lo + 8] for j in range(NT)], axis=1)
                        for g in range(NG)], axis=0)
                    orr[s2, 2 * t + o_] = (xx + o).astype(BF16)

                def a(t, gs):
                    for g in gs:
                        stage_a(g, P[t], P[t + 1], sb, cb.at[0])

                def bq(qs):
                    for q in qs:
                        stage_b(q, cb.at[zero], z16, 0, 0)

                def c(t, nxt):
                    nq = 2 * NM
                    for q in range(nq):
                        stage_c(q % NM, z16[q // NM], gt16, q // NM, None)
                        if nxt:
                            a(t + 1, range(q * NG // nq, (q + 1) * NG // nq))

                ds(0); a(0, range(0, 4)); ds(1); a(0, range(4, 8)); ds(2); a(0, range(8, 12))
                ds(3); bq(range(12)); ds(4)
                c(0, True)
                ds(5); bq(range(12)); dr(0, 0); dr(0, 1)
                c(1, True)
                ds(6); bq(range(12)); dr(1, 0); dr(1, 1)
                c(2, False)
                ds(7); dr(2, 0); dr(2, 1); ds(8); ds(9)
                return s3n

            s3 = lax.fori_loop(0, NI, body2, 0)
            s_out(NI - 1, (NI - 1) % 3).start()
            r_out(NI - 1, (NI - 1) & 1).start()
            s_out(NI - 2, (NI - 2) % 3).wait()
            r_out(NI - 2, (NI - 2) & 1).wait()
            s_out(NI - 1, (NI - 1) % 3).wait()
            r_out(NI - 1, (NI - 1) & 1).wait()

        if do2:
            pl.run_scoped(
                pass2,
                pltpu.VMEM((3, 2 * SA, C, 512), BF16),
                pltpu.VMEM((7, 48, 8, 128), U32),
                pltpu.VMEM((2, 2 * RA, C, 512), BF16),
                pltpu.VMEM((2, 48, 8, 128), U32),
                pltpu.VMEM((1, 8, C, 128), F32),
                pltpu.VMEM((2, C // 2, 512), U32),
                pltpu.VMEM((2, E // 2, 512), U32),
            )

    @jax.jit
    def f(x, dw, w1, w2, grn_gamma, grn_beta):
        xt = x.reshape(512, NT, 128, NG, 8).transpose(0, 3, 1, 4, 2).reshape(NP, 2, NG * NT, 8, 128)
        xn = x.reshape(512, 512, C).transpose(0, 2, 1)
        vm = pl.BlockSpec(memory_space=pltpu.VMEM)
        hb = pl.BlockSpec(memory_space=pl.ANY)
        o = pl.pallas_call(
            kern,
            out_shape=jax.ShapeDtypeStruct(xn.shape, xn.dtype),
            in_specs=[hb, hb, vm, vm, vm, vm, vm],
            out_specs=hb,
            scratch_shapes=[
                pltpu.VMEM((2 * NS, E // 2, 512), U32),
                pltpu.VMEM((1, WB, 128), U32),
                pltpu.VMEM((8, 128), F32),
                pltpu.VMEM((C // 2, E), U32),
                pltpu.VMEM((C, 128), F32),
                pltpu.SMEM((1,), jnp.int32),
                pltpu.SemaphoreType.DMA((12,)),
            ],
            compiler_params=pltpu.CompilerParams(vmem_limit_bytes=128 << 20, flags=flags),
            name="cnx",
        )(xt, xn, dw, w1, w2.T, grn_gamma, grn_beta)
        return o.transpose(0, 2, 1).reshape(x.shape)
    return f


pallas_standalone__modern_conv_block_convnext_v2__vision_kernel = build(U=4)
```

```python
import math

import jax
import jax.numpy as jnp
from jax import lax
import jax.experimental.pallas as pl
import jax.experimental.pallas.tpu as pltpu

F32, BF16, U32 = jnp.float32, jnp.bfloat16, jnp.uint32
C, E, NG, NT = 96, 384, 12, 4
NP = 256
_C0 = math.sqrt(2.0 / math.pi)
_K = (_C0 * 0.044715) ** (1.0 / 3.0)
_B = _C0 / _K
_GS = 0.5 / _K
W1, S1, S2, RS, W2, AN, AW, AC = 0, 192, 264, 336, 352, 496, 504, 600
WB = AC + E


def build(U=4, MC=64, SA=5, RA=3, do1=True, do2=True, order1="cbagp", flags=None, mst=False, NC=2, LA=2, LP=4, LK=3, QB=10, GC=1, cut=0, G2=6, lag=0, DC=192, DD=150, DV=300, p5="C0 B0 V1 S V2 R0 B1 V2 C1 Q V1 S V2 R1 Z0 V2 S Z1 V2", p6=None):
    NB = NP // U
    NI = NP // (SA + RA)
    NS, NR = SA * NI, RA * NI
    NM = E // MC
    plan = (p5, p5, p6 or p5 + ' S')

    def kern(x_hbm, xn_hbm, dw_ref, w1_ref, w2t_ref, gam_ref, bet_ref, o_hbm,
             G, wb, bias, zs, sem):
        x32 = x_hbm.bitcast(U32)
        G16 = G.bitcast(BF16)
        for j in range(1 + NT):
            zs[j] = 0
        lane = lax.broadcasted_iota(jnp.int32, (8, 128), 1)

        def in_hi(p0, n, dst, s):
            return pltpu.make_async_copy(x32.at[pl.ds(p0 - 1, n), 1], dst.at[:, pl.ds(0, 48), pl.ds(0, 4)], s)

        def in_lo(p0, n, dst, s):
            return pltpu.make_async_copy(x32.at[pl.ds(p0, n), 0], dst.at[:, pl.ds(0, 48), pl.ds(4, 4)], s)

        def taps():
            d = dw_ref[...].astype(F32)
            rows = [d[i, j:j + 1, :] for i in range(3) for j in range(3)]
            dm = jnp.concatenate(rows + [jnp.zeros((128 - 9, C), F32)], axis=0)
            dm = jnp.concatenate([dm, jnp.zeros((128, 128 - C), F32)], axis=1)
            dt = dm.T[:C]
            return [jnp.broadcast_to(dt[:, t:t + 1], (C, 128)) for t in range(9)]

        def prep_weights():
            tp = taps()
            r = lax.broadcasted_iota(jnp.int32, (C, 128), 0)
            k = lax.broadcasted_iota(jnp.int32, (C, 128), 1)
            diag = (r & 7) == (k & 7)
            slot = k >> 3
            outs = []
            for o in range(2):
                a = jnp.zeros((C, 128), F32)
                for i in range(3):
                    ri = i + o
                    for j in range(3):
                        s = ((ri >> 1) * 3 + j) * 2 + (ri & 1)
                        a = jnp.where(diag & (slot == s), tp[i * 3 + j], a)
                outs.append(a)
            for g in range(NG):
                wb[0, AW + 8 * g:AW + 8 * g + 8] = pltpu.bitcast(
                    jnp.concatenate([outs[0][8 * g:8 * g + 8], outs[1][8 * g:8 * g + 8]], axis=0).astype(BF16), U32)
            w = w1_ref[...].astype(F32)
            w = w - jnp.sum(w, axis=0, keepdims=True) * (1.0 / C)
            w = jnp.concatenate([w, jnp.zeros((128 - C, E), F32)], axis=0)
            wb[0, W1:W1 + E // 2] = pltpu.bitcast(w.T.astype(BF16), U32)

        def stage_p(g, new, sb):
            v = [new[4 * g + j] for j in range(NT)]
            r = [pltpu.roll(t, 1, 1) for t in v]
            l = [pltpu.roll(t, 127, 1) for t in v]
            z = jnp.zeros((8, 128), U32)
            for j in range(NT):
                if mst:
                    pltpu.store(sb.at[0, 4 * g + j], r[j], mask=lane != 0)
                    pltpu.store(sb.at[1, 4 * g + j], l[j], mask=lane != 127)
                    if j > 0:
                        pltpu.store(sb.at[0, 4 * g + j], r[j - 1], mask=lane == 0)
                    if j < NT - 1:
                        pltpu.store(sb.at[1, 4 * g + j], l[j + 1], mask=lane == 127)
                else:
                    sb[0, 4 * g + j] = jnp.where(lane == 0, r[j - 1] if j > 0 else z, r[j])
                    sb[1, 4 * g + j] = jnp.where(lane == 127, l[j + 1] if j < NT - 1 else z, l[j])

        def stage_a(g, old, new, s_old, s_new, c_out):
            cols = [jnp.concatenate([s_old[0, t], old[t], s_old[1, t], s_new[0, t], new[t], s_new[1, t]], axis=0)
                    for t in range(4 * g, 4 * g + NT)]
            rhs = pltpu.bitcast(jnp.concatenate(cols, axis=1), BF16)
            res = jnp.dot(pltpu.bitcast(wb[0, AW + 8 * g:AW + 8 * g + 8], BF16)[:, :C], rhs, preferred_element_type=F32)
            for o in range(2):
                for j in range(NT):
                    c_out[(4 * o + j) * C + 8 * g:(4 * o + j) * C + 8 * g + 8] = res[8 * o:8 * o + 8, 128 * j:128 * j + 128]

        def tree(v):
            while len(v) > 1:
                v = [v[i] + v[i + 1] if i + 1 < len(v) else v[i] for i in range(0, len(v), 2)]
            return v[0]

        def stage_b1(q, c_in, zero):
            s1 = s2 = None
            for g in range(NG):
                c = c_in[q * C + 8 * g:q * C + 8 * g + 8]
                s1 = c if s1 is None else s1 + c
                s2 = c * c if s2 is None else s2 + c * c
            wb[zero, S1 + 9 * q:S1 + 9 * q + 8] = pltpu.bitcast(s1, U32)
            wb[zero, S2 + 9 * q:S2 + 9 * q + 8] = pltpu.bitcast(s2, U32)

        def stage_b2(e, zero):
            s1 = tree([pltpu.bitcast(wb[0, pl.ds(S1 + i, 8, stride=9), :], F32) for i in range(8)])
            s2 = tree([pltpu.bitcast(wb[0, pl.ds(S2 + i, 8, stride=9), :], F32) for i in range(8)])
            v = jnp.maximum(s2 - s1 * s1 * (1.0 / C), 0.0)
            wb[zero, RS + 8 * e:RS + 8 * e + 8] = pltpu.bitcast(lax.rsqrt(v * (1.0 / (C * _K * _K)) + 1e-5 / (_K * _K)), U32)

        def stage_b3(q, e, c_in, z16, zrow):
            o, j = divmod(q, NT)
            z16[pl.ds(zrow + o, 1), :, 128 * j:128 * j + 128] = (c_in[q * C:(q + 1) * C] * pltpu.bitcast(wb[0, RS + 8 * e + q:RS + 8 * e + q + 1], F32))[None].astype(BF16)

        def mm1(m, rhs, n=1):
            lhs = pltpu.bitcast(wb[0, W1 + m * MC // 2:W1 + (m + n) * MC // 2], BF16)[:, :C]
            return jnp.dot(lhs, rhs, preferred_element_type=F32)

        def act(m, z, g16, grow, acc):
            gl = z + z * jnp.tanh(z * (z * z + _B))
            g16[pl.ds(grow, 1), m * MC:(m + 1) * MC, :] = gl[None].astype(BF16)
            if acc is None:
                return gl
            else:
                sq = gl * gl
                sq = (sq[:, 0:128] + sq[:, 128:256]) + (sq[:, 256:384] + sq[:, 384:512])
                rows = slice(AC + m * MC, AC + (m + 1) * MC)
                wb[acc, rows] = pltpu.bitcast(pltpu.bitcast(wb[acc, rows], F32) + sq, U32)

        XN = U + 2

        def pass1(xb, sbs, cbs, zb, raw):
            z16 = zb.bitcast(BF16)

            def blk(b, slot, nh=XN, nl=XN):
                return [in_hi(b * U + 3, nh, xb.at[slot, pl.ds(0, nh)], sem.at[slot]),
                        in_lo(b * U + 3, nl, xb.at[slot, pl.ds(0, nl)], sem.at[2 + slot])]

            def end_blk(b):
                n = NP - (b * U + 3)
                return blk(b, b & 1, n + 1, n), n

            pins, pend = {}, {}

            def run_slot(t, xp, zero, grow, lo):
                p, q = divmod(t, 12)
                if t - LK in pins:
                    xb[zero, 0, 48] = pltpu.bitcast(pins[t - LK], U32)
                for st in order1:
                    if st == "c" and p >= lo and q % GC == 0:
                        zz = mm1(q % NM, z16[2 * (p & 1) + q // NM], GC)
                        for k in range(GC):
                            z = zz[k * MC:(k + 1) * MC]
                            pins[t + k] = z[0:8, 0:128]
                            if t + k >= 12 * U - NC:
                                raw[t + k - (12 * U - NC)] = z
                            else:
                                pend[t + k] = z
                    if st == "g" and p >= lo:
                        pg, qg = divmod(t - NC, 12)
                        act(qg % NM, raw[t] if t < NC else pend.pop(t - NC), G16, grow(pg) + qg // NM, zero)
                    if st == "b":
                        if q < 8 and p + 2 >= lo:
                            stage_b1(q, cbs[(p + 2) & 3].at[zero], zero)
                        if q == QB and p + 2 >= lo:
                            stage_b2(p & 1, zero)
                        if q >= 8 and p + 1 >= lo:
                            for k in range(2 * (q - 8), 2 * (q - 8) + 2):
                                stage_b3(k, (p + 1) & 1, cbs[(p + 1) & 3].at[zero], z16, 2 * ((p + 1) & 1) + zero)
                    if st == "p":
                        pp, g = divmod(t + 48 + LP, 12)
                        if pp >= lo:
                            stage_p(g, xp(pp), sbs.at[pp & 1] if False else sbs[pp & 3].at[0])
                    if st == "a":
                        pa, g = divmod(t + 36 + LA, 12)
                        if pa >= lo:
                            stage_a(g, xp(pa), xp(pa + 1), sbs[pa & 3].at[zero], sbs[(pa + 1) & 3].at[zero], cbs[pa & 3].at[0])

            pa_ = in_hi(1, 4, xb.at[1, pl.ds(1, 4)], sem.at[1])
            pb_ = in_lo(0, 5, xb.at[1, pl.ds(0, 5)], sem.at[3])
            pa_.start()
            pb_.start()
            for c_ in blk(0, 0):
                c_.start()
            prep_weights()
            wb[0, AC:AC + E] = jnp.zeros((E, 128), U32)
            raw[...] = jnp.zeros_like(raw)
            if mst:
                for sb in sbs:
                    for g in range(NG):
                        sb[0, 0, 4 * g] = jnp.zeros((8, 128), U32)
                        sb[0, 1, 4 * g + 3] = jnp.zeros((8, 128), U32)
            pa_.wait()
            pb_.wait()
            xb[1, 0, 0:48, 0:4, :] = jnp.zeros((48, 4, 128), U32)
            for t in range(-48 - LP, 0):
                run_slot(t, lambda p: xb.at[1, p], zs[0], None, 0)

            def drain(row):
                for k in range(NC):
                    act(NM - NC + k, raw[k], G16, row, 0)

            def body1(b, _):
                slot = b & 1
                zero = zs[0]

                @pl.when(b < NB - 2)
                def _():
                    for c_ in blk(b, slot):
                        c_.wait()

                @pl.when(b < NB - 3)
                def _():
                    for c_ in blk(b + 1, 1 - slot):
                        c_.start()

                @pl.when(b >= NB - 3)
                def _():
                    for e in (NB - 2, NB - 1):
                        @pl.when(b == e)
                        def _():
                            cs, n = end_blk(e)
                            for c_ in cs:
                                c_.wait()
                            xb[e & 1, n, 0:48, 4:8, :] = jnp.zeros((48, 4, 128), U32)

                        @pl.when(b == e - 1)
                        def _():
                            for c_ in end_blk(e)[0]:
                                c_.start()

                grow = lambda p: 2 * jnp.maximum(b * U + p - NR, 0)
                for t in range(12 * U):
                    run_slot(t, lambda p: xb.at[slot, p - 3], zero, grow, -99)
                return 0

            lax.fori_loop(0, NB, body1, 0)
            drain(2 * NS - 1 - cut)

            ss = jnp.sum(pltpu.bitcast(wb[0, AC:AC + E], F32).T, axis=0, keepdims=True)
            gx = jnp.sqrt(ss * (_GS * _GS) + 1e-6)
            nx = gx / (jnp.sum(gx, axis=1, keepdims=True) * (1.0 / E) + 1e-6)
            gam = gam_ref[...].astype(F32).reshape(1, E)
            bet = bet_ref[...].astype(F32).reshape(1, E)
            w2 = w2t_ref[...].astype(F32)
            w2s = pltpu.bitcast((w2 * ((gam * nx + 1.0) * _GS)).astype(BF16), U32)
            for k in range(3):
                wb[0, W2 + 48 * k:W2 + 48 * k + 48] = w2s[:, 128 * k:128 * k + 128]
            bias[0] = jnp.broadcast_to(jnp.sum(w2 * bet, axis=1, keepdims=True), (C, 128))

        if do1:
            pl.run_scoped(
                pass1,
                pltpu.VMEM((2, XN, 49, 8, 128), U32),
                [pltpu.VMEM((1, 2, 48, 8, 128), U32)] * 4,
                [pltpu.VMEM((1, 8 * C, 128), F32)] * 4,
                pltpu.VMEM((4, C // 2, 512), U32),
                pltpu.VMEM((max(NC, 1), MC, 512), F32),
            )

        if not do1:
            bias[0] = jnp.zeros((C, 128), F32)
        def pass2(xs, xr, tb, cb, zb, gt):
            z16 = zb.bitcast(BF16)
            gt16 = gt.bitcast(BF16)
            RR, SR = 2 * RA, 2 * SA

            def s_in(i, slot):
                return pltpu.make_async_copy(xn_hbm.at[pl.ds(2 * NR + SR * i, SR)], xs.at[slot], sem.at[4 + slot])

            def s_out(i, slot):
                return pltpu.make_async_copy(xs.at[slot], o_hbm.at[pl.ds(2 * NR + SR * i, SR)], sem.at[7 + slot])

            def r_in(i):
                return pltpu.make_async_copy(xn_hbm.at[pl.ds(RR * i, RR)], xr.at[pl.ds(RR * (i & 3), RR)], sem.at[i & 3])

            def r_out(i):
                return pltpu.make_async_copy(xr.at[pl.ds(RR * (i & 3), RR)], o_hbm.at[pl.ds(RR * i, RR)], sem.at[10 + (i & 3)])

            def anchor(v, zero):
                wb[zero, AN:AN + 8] = pltpu.bitcast(v[-8:, -128:], U32)

            def stage_v(g, rows, c_out, zero):
                w = [tb[0, C * t + 8 * g:C * t + 8 * g + 8] for t in range(9)]
                d = [None if r is None else r[8 * g:8 * g + 8, :].astype(F32) for r in rows]
                z = jnp.zeros((8, 128), F32)
                ms, rs = [], []
                for o in range(2):
                    part = [[tree([d[o + i][:, 128 * j:128 * j + 128] * w[3 * i + dx] for i in range(3) if d[o + i] is not None])
                             for j in range(NT)] for dx in range(3)]
                    r = [pltpu.roll(t, 1, 1) for t in part[0]]
                    l = [pltpu.roll(t, 127, 1) for t in part[2]]
                    for j in range(NT):
                        res = (part[1][j] + jnp.where(lane == 0, r[j - 1] if j > 0 else z, r[j])
                               + jnp.where(lane == 127, l[j + 1] if j < NT - 1 else z, l[j]))
                        c_out[(4 * o + j) * C + 8 * g:(4 * o + j) * C + 8 * g + 8] = res
                        rs.append(res)
                    ms += part[1]
                res = tree(rs)
                pin = tree(ms) if lag else res
                tb[zero, 9 * C:9 * C + 8] = pin
                xr[4 * RR + zero, 0:8, 0:256] = jnp.concatenate([pin, pin], axis=1).astype(BF16)
                return res

            r_in(0).start()
            r_in(1).start()
            s_in(0, 0).start()
            for t, v in enumerate(taps()):
                tb[0, C * t:C * t + C] = v
            r_in(0).wait()
            for p in range(2):
                for g in range(NG):
                    stage_v(g, [None if r < 0 else xr.at[r] for r in range(2 * p - 1, 2 * p + 3)], cb.at[p], zs[0])
            for q in range(8):
                stage_b1(q, cb.at[0], 0)
            stage_b2(0, 0)
            for q in range(8):
                stage_b3(q, 0, cb.at[0], z16, 0)

            def mm2(rhs, xrow, h, zj):
                o = []
                for j in (2 * h, 2 * h + 1):
                    lhs = jnp.concatenate([wb[zj[j], W2 + 48 * k:W2 + 48 * k + 48] for k in range(3)], axis=1)
                    o.append(jnp.dot(pltpu.bitcast(lhs, BF16), rhs[:, 128 * j:128 * j + 128], preferred_element_type=F32) + bias[zj[j]])

                def fin():
                    res = jnp.concatenate(o, axis=1) + xrow[:, 256 * h:256 * h + 256].astype(F32)
                    xrow[:, 256 * h:256 * h + 256] = res.astype(BF16)
                    return res
                return fin

            def body2(i, s3):
                zero = zs[0]
                zj = [zs[1 + j] for j in range(NT)]
                s3p = jnp.where(s3 == 0, 2, s3 - 1)
                s3n = jnp.where(s3 == 2, 0, s3 + 1)

                @pl.when(i >= 1)
                def _():
                    s_out(i - 1, s3p).start()
                    r_out(i - 1).start()

                @pl.when(i >= 2)
                def _():
                    s_out(i - 2, s3n).wait()
                    r_out(i - 2).wait()

                @pl.when(i < NI - 1)
                def _():
                    r_in(i + 2).start()
                    s_in(i + 1, s3n).start()

                r_in(i + 1).wait()
                s_in(i, s3).wait()

                xrow = lambda r: xr.at[RR * ((i + r // RR) & 3) + r % RR]
                late = []
                now = [0]

                def flush(n):
                    for d, f in [w for w in late if w[0] <= now[0]]:
                        anchor(f(), zero)
                    late[:] = [w for w in late if w[0] > now[0]]
                    now[0] += n

                ns = 0
                for k in range(RA):
                    e = (i * RA + k) & 1
                    nv = 0
                    for tok in plan[k].split():
                        if tok[0] == "C":
                            o = int(tok[1])
                            for m in range(0, NM, G2):
                                flush(G2 * MC)
                                zz = mm1(m, z16[o], G2)
                                for u in range(G2):
                                    late.append((now[0] - (G2 - 1 - u) * MC + DC, lambda m=m, u=u, zz=zz, o=o: act(
                                        m + u, zz[u * MC:(u + 1) * MC], gt16, zero, None)))
                        elif tok[0] == "S":
                            for h in range(2):
                                flush(96 + 96 * h)
                                late.append((now[0] + 96 * (1 - h) + DD, mm2(G16.at[SR * i + ns], xs.at[s3, ns], h, zj)))
                            ns += 1
                        elif tok[0] == "R":
                            for h in range(2):
                                flush(96 + 96 * h)
                                late.append((now[0] + 96 * (1 - h) + DD, mm2(gt16.at[0], xrow(2 * k + int(tok[1])), h, zj)))
                        elif tok[0] == "V":
                            for g in range(nv, nv + int(tok[1])):
                                v = stage_v(g, [xrow(r) for r in range(2 * k + 3, 2 * k + 7)], cb.at[e], zero)
                                late.append((now[0] + DV, lambda v=v: v))
                            nv += int(tok[1])
                        elif tok[0] == "B":
                            for q in range(4 * int(tok[1]), 4 * int(tok[1]) + 4):
                                stage_b1(q, cb.at[1 - e], zero)
                        elif tok[0] == "Q":
                            stage_b2(0, zero)
                        elif tok[0] == "Z":
                            for q in range(4 * int(tok[1]), 4 * int(tok[1]) + 4):
                                stage_b3(q, 0, cb.at[1 - e], z16, zero)
                    assert nv == NG
                assert ns == SR
                now[0] = 1 << 30
                flush(0)
                return s3n

            lax.fori_loop(0, NI, body2, 0)
            s_out(NI - 1, (NI - 1) % 3).start()
            r_out(NI - 1).start()
            for i in (NI - 2, NI - 1):
                s_out(i, i % 3).wait()
                r_out(i).wait()

        if do2:
            pl.run_scoped(
                pass2,
                pltpu.VMEM((3, 2 * SA, C, 512), BF16),
                pltpu.VMEM((8 * RA + 1, C, 512), BF16),
                pltpu.VMEM((1, 9 * C + 8, 128), F32),
                pltpu.VMEM((2, 8 * C, 128), F32),
                pltpu.VMEM((2, C // 2, 512), U32),
                pltpu.VMEM((1, E // 2, 512), U32),
            )
        else:
            def keep(buf):
                buf[...] = G16[zs[0], 0:16]
                pltpu.sync_copy(buf, o_hbm.at[0, pl.ds(0, 16)])
            pl.run_scoped(keep, pltpu.VMEM((16, 512), BF16))

    @jax.jit
    def f(x, dw, w1, w2, grn_gamma, grn_beta):
        xt = x.reshape(512, NT, 128, NG, 8).transpose(0, 3, 1, 4, 2).reshape(NP, 2, NG * NT, 8, 128)
        xn = x.reshape(512, 512, C).transpose(0, 2, 1)
        vm = pl.BlockSpec(memory_space=pltpu.VMEM)
        hb = pl.BlockSpec(memory_space=pl.ANY)
        o = pl.pallas_call(
            kern,
            out_shape=jax.ShapeDtypeStruct(xn.shape, xn.dtype),
            in_specs=[hb, hb, vm, vm, vm, vm, vm],
            out_specs=hb,
            scratch_shapes=[
                pltpu.VMEM((2 * NS - cut, E // 2, 512), U32),
                pltpu.VMEM((1, WB, 128), U32),
                pltpu.VMEM((1, C, 128), F32),
                pltpu.SMEM((1 + NT,), jnp.int32),
                pltpu.SemaphoreType.DMA((14,)),
            ],
            compiler_params=pltpu.CompilerParams(vmem_limit_bytes=128 << 20, flags=flags, disable_bounds_checks=True),
            name="cnx",
        )(xt, xn, dw, w1, w2.T, grn_gamma, grn_beta)
        return o.transpose(0, 2, 1).reshape(x.shape)
    return f


pallas_standalone__modern_conv_block_convnext_v2__vision_kernel = build(U=4)
```

```python
import functools
import math

import jax
import jax.numpy as jnp
from jax import lax
import jax.experimental.pallas as pl
import jax.experimental.pallas.tpu as pltpu

F32, BF16, U32 = jnp.float32, jnp.bfloat16, jnp.uint32
C, E, NG, NT = 96, 384, 12, 4
NP = 256
_C0 = math.sqrt(2.0 / math.pi)
_K = (_C0 * 0.044715) ** (1.0 / 3.0)
_B = _C0 / _K
_GS = 0.5 / _K
W1, S1, S2, RS, W2, AN, AW, AC = 0, 192, 264, 336, 352, 496, 504, 600
WB = AC + E


def build(U=8, MC=64, SA=5, RA=3, do1=True, do2=True, order1="cabgp", flags=None, mst=False, NC=2, LA=2, LP=4, LK=3, LB=2, pb1=1, QA=8, QB=9, il=(), cut=0, nodma=0, NGT=1, NSB=16, RT=0, two=False, had=False, DB=200, DQ=200, lag=0, DC=192, DD=150, DV=500, p5="C0 B01 V1 B23 S V1 B45 V1 B67 R0 V2 C1 Q V1 S V2 R1 Z01 V1 Z23 V1 S Z45 V1 Z67 V1", p6=None):
    NB = NP // U
    NI = NP // (SA + RA)
    NS, NR = SA * NI, RA * NI
    NM = E // MC
    plan = (p5, p5, p6 or p5 + ' S')

    def kern(x_hbm, xn_hbm, dw_ref, w1_ref, w2t_ref, gam_ref, bet_ref, o_hbm,
             G, wb, bias, zs, sem):
        x32 = x_hbm.bitcast(U32)
        G16 = G.bitcast(BF16)
        for j in range(1 + NT):
            zs[j] = 0
        lane = lax.broadcasted_iota(jnp.int32, (8, 128), 1)

        def in_hi(p0, n, dst, s):
            return pltpu.make_async_copy(x32.at[pl.ds(p0 - 1, n), 1], dst.at[:, pl.ds(0, 48), pl.ds(0, 4)], s)

        def in_lo(p0, n, dst, s):
            return pltpu.make_async_copy(x32.at[pl.ds(p0, n), 0], dst.at[:, pl.ds(0, 48), pl.ds(4, 4)], s)

        def taps():
            d = dw_ref[...].astype(F32)
            rows = [d[i, j:j + 1, :] for i in range(3) for j in range(3)]
            dm = jnp.concatenate(rows + [jnp.zeros((128 - 9, C), F32)], axis=0)
            dm = jnp.concatenate([dm, jnp.zeros((128, 128 - C), F32)], axis=1)
            dt = dm.T[:C]
            return [jnp.broadcast_to(dt[:, t:t + 1], (C, 128)) for t in range(9)]

        def prep_weights():
            tp = taps()
            r = lax.broadcasted_iota(jnp.int32, (C, 128), 0)
            k = lax.broadcasted_iota(jnp.int32, (C, 128), 1)
            diag = (r & 7) == (k & 7)
            slot = k >> 3
            outs = []
            for o in range(2):
                a = jnp.zeros((C, 128), F32)
                for i in range(3):
                    ri = i + o
                    for j in range(3):
                        s = ((ri >> 1) * 3 + j) * 2 + (ri & 1)
                        a = jnp.where(diag & (slot == s), tp[i * 3 + j], a)
                outs.append(a)
            for g in range(NG):
                wb[0, AW + 8 * g:AW + 8 * g + 8] = pltpu.bitcast(
                    jnp.concatenate([outs[0][8 * g:8 * g + 8], outs[1][8 * g:8 * g + 8]], axis=0).astype(BF16), U32)
            w = w1_ref[...].astype(F32)
            w = w - jnp.sum(w, axis=0, keepdims=True) * (1.0 / C)
            w = jnp.concatenate([w, jnp.zeros((128 - C, E), F32)], axis=0)
            wb[0, W1:W1 + E // 2] = pltpu.bitcast(w.T.astype(BF16), U32)

        def stage_p(g, new, sb):
            v = [new[4 * g + j] for j in range(NT)]
            r = [pltpu.roll(t, 1, 1) for t in v]
            l = [pltpu.roll(t, 127, 1) for t in v]
            z = jnp.zeros((8, 128), U32)
            for j in range(NT):
                if mst:
                    pltpu.store(sb.at[0, j], r[j], mask=lane != 0)
                    pltpu.store(sb.at[1, j], l[j], mask=lane != 127)
                    if j > 0:
                        pltpu.store(sb.at[0, j], r[j - 1], mask=lane == 0)
                    if j < NT - 1:
                        pltpu.store(sb.at[1, j], l[j + 1], mask=lane == 127)
                else:
                    sb[0, j] = jnp.where(lane == 0, r[j - 1] if j > 0 else z, r[j])
                    sb[1, j] = jnp.where(lane == 127, l[j + 1] if j < NT - 1 else z, l[j])

        def stage_a(g, old, new, s_old, s_new, c_out):
            cols = [jnp.concatenate([s_old[0, j], old[4 * g + j], s_old[1, j], s_new[0, j], new[4 * g + j], s_new[1, j]], axis=0)
                    for j in range(NT)]
            rhs = pltpu.bitcast(jnp.concatenate(cols, axis=1), BF16)
            res = jnp.dot(pltpu.bitcast(wb[0, AW + 8 * g:AW + 8 * g + 8], BF16)[:, :C], rhs, preferred_element_type=F32)
            for o in range(2):
                for j in range(NT):
                    c_out[(4 * o + j) * C + 8 * g:(4 * o + j) * C + 8 * g + 8] = res[8 * o:8 * o + 8, 128 * j:128 * j + 128]

        def tree(v):
            while len(v) > 1:
                v = [v[i] + v[i + 1] if i + 1 < len(v) else v[i] for i in range(0, len(v), 2)]
            return v[0]

        def stage_b1(q, c_in, zero, defer=False):
            s1 = s2 = None
            for g in range(NG):
                c = c_in[q * C + 8 * g:q * C + 8 * g + 8]
                s1 = c if s1 is None else s1 + c
                s2 = c * c if s2 is None else s2 + c * c

            def put():
                wb[zero, S1 + 9 * q:S1 + 9 * q + 8] = pltpu.bitcast(s1, U32)
                wb[zero, S2 + 9 * q:S2 + 9 * q + 8] = pltpu.bitcast(s2, U32)
            return put if defer else put()

        def stage_b2(c_io, zero):
            s1 = tree([pltpu.bitcast(wb[0, pl.ds(S1 + i, 8, stride=9), :], F32) for i in range(8)])
            s2 = tree([pltpu.bitcast(wb[0, pl.ds(S2 + i, 8, stride=9), :], F32) for i in range(8)])
            v = jnp.maximum(s2 - s1 * s1 * (1.0 / C), 0.0)
            r = lax.rsqrt(v * (1.0 / (C * _K * _K)) + 1e-5 / (_K * _K))
            if c_io is not None:
                c_io[8 * C:8 * C + 8] = r

            def put():
                wb[zero, RS:RS + 8] = pltpu.bitcast(r, U32)
            return put

        def stage_b3(q, c_in, z16, zrow, rw=False):
            o, j = divmod(q, NT)
            r = pltpu.bitcast(wb[0, RS + q:RS + q + 1], F32) if rw else c_in[8 * C + q:8 * C + q + 1]
            z16[pl.ds(zrow + o, 1), :, 128 * j:128 * j + 128] = (c_in[q * C:(q + 1) * C] * r)[None].astype(BF16)

        def mm1(m, rhs, n=1):
            lhs = pltpu.bitcast(wb[0, W1 + m * MC // 2:W1 + (m + n) * MC // 2], BF16)[:, :C]
            return jnp.dot(lhs, rhs, preferred_element_type=F32)

        held, nost = [], [0]

        def act(m, z, g16, grow, acc, hold=False):
            gl = z + z * jnp.tanh(z * (z * z + _B))
            if not nost[0]:
                g16[pl.ds(grow, 1), m * MC:(m + 1) * MC, :] = gl[None].astype(BF16)
            if acc is None:
                return gl
            else:
                sq = gl * gl
                sq = (sq[:, 0:128] + sq[:, 128:256]) + (sq[:, 256:384] + sq[:, 384:512])
                if hold:
                    held.append(sq)
                    for k in il[1:]:
                        wb[acc, AN:AN + 8] = pltpu.bitcast(sq[8 * k:8 * k + 8], U32)
                    return
                if held:
                    sq = sq + held.pop()
                rows = slice(AC + m * MC, AC + (m + 1) * MC)
                wb[acc, rows] = pltpu.bitcast(pltpu.bitcast(wb[acc, rows], F32) + sq, U32)

        XN = U + 2
        NE = -(-(NP - U - 4) // U)

        def pass1(xb, sbs, cbs, zb, raw):
            z16 = zb.bitcast(BF16)

            def blk(b, slot, nh=XN, nl=XN):
                return [in_hi(b * U + 3, nh, xb.at[slot, pl.ds(0, nh)], sem.at[slot]),
                        in_lo(b * U + 3, nl, xb.at[slot, pl.ds(0, nl)], sem.at[2 + slot])]

            def end_blk(b):
                n = NP - (b * U + 3)
                return blk(b, b & 1, n + 1, n), n

            sring = lambda n, zero: sbs[(n & 15) % NSB].at[zero + (n & 15) // NSB]
            pins, pend = {}, {}
            om = (lambda q: (q & 1, q >> 1)) if il else (lambda q: divmod(q, NM))

            def run_slot(t, xp, zero, grow, lo):
                p, q = divmod(t, 12)
                if t - LK in pins:
                    xb[zero, 0, 48] = pltpu.bitcast(pins[t - LK], U32)
                if t - LB in pins and (q >= 8 or pb1):
                    cbs[(p + (2 if q < 8 else 1)) & 3][0, 8 * C + 8:8 * C + 16] = pins[t - LB]
                for st in order1:
                    if st == "c" and p >= lo:
                        o, m = om(q)
                        z = mm1(m, z16[2 * (p & 1) + o])
                        pins[t] = z[0:8, 0:128]
                        if t == 12 * U - 1:
                            raw[0] = z
                        else:
                            pend[t] = z
                    if st == "g" and p >= lo:
                        for tg in [-1] * (t == RT) + list(range(max(t - NC, 0), t if t == 12 * U - 1 else t - NC + 1)):
                            pg, qg = divmod(tg, 12)
                            o, m = om(qg)
                            act(m, raw[0] if tg < 0 else pend.pop(tg), G16, grow(pg) + o, zero,
                                hold=il and o == 0 and tg != 12 * U - 2)
                    if st == "b":
                        if q < 8 and p + 2 >= lo:
                            stage_b1(q, cbs[(p + 2) & 3].at[zero], zero)
                        if q == QA and p + 2 >= lo:
                            pend["r"] = stage_b2(cbs[(p + 2) & 3].at[0], zero)
                        if q == QB and p + 2 >= lo:
                            pend.pop("r")()
                        if q >= 8 and p + 1 >= lo:
                            for k in range(2 * (q - 8), 2 * (q - 8) + 2):
                                stage_b3(k, cbs[(p + 1) & 3].at[zero], z16, 2 * ((p + 1) & 1) + zero)
                    if st == "p":
                        pp, g = divmod(t + 48 + LP, 12)
                        if pp >= lo:
                            stage_p(g, xp(pp), sring(12 * pp + g, 0))
                    if st == "a":
                        pa, g = divmod(t + 36 + LA, 12)
                        if pa >= lo:
                            stage_a(g, xp(pa), xp(pa + 1), sring(12 * pa + g, zero), sring(12 * pa + 12 + g, zero), cbs[pa & 3].at[0])

            pa_ = in_hi(1, 4, xb.at[1, pl.ds(1, 4)], sem.at[1])
            pb_ = in_lo(0, 5, xb.at[1, pl.ds(0, 5)], sem.at[3])
            pa_.start()
            pb_.start()
            for c_ in blk(0, 0):
                c_.start()
            prep_weights()
            wb[0, AC:AC + E] = jnp.zeros((E, 128), U32)
            raw[...] = jnp.zeros_like(raw)
            if mst:
                for sb in sbs:
                    for g in range(16 // NSB):
                        sb[g, 0, 0] = jnp.zeros((8, 128), U32)
                        sb[g, 1, 3] = jnp.zeros((8, 128), U32)
            pa_.wait()
            pb_.wait()
            xb[1, 0, 0:48, 0:4, :] = jnp.zeros((48, 4, 128), U32)
            for t in range(-48 - LP, 0):
                run_slot(t, lambda p: xb.at[1, p], zs[0], None, 0)

            def drain(row):
                act(NM - 1, raw[0], G16, row, 0)

            def body1(b, _):
                slot = b & 1
                zero = zs[0]

                @pl.when(b < NE)
                def _():
                    for c_ in blk(b, slot):
                        c_.wait()

                @pl.when(b < NE - 1)
                def _():
                    for c_ in blk(b + 1, 1 - slot):
                        c_.start()

                @pl.when(b >= NE - 1)
                def _():
                    for e in range(NE, NB):
                        @pl.when(b == e)
                        def _():
                            cs, n = end_blk(e)
                            for c_ in cs:
                                c_.wait()
                            xb[e & 1, n, 0:48, 4:8, :] = jnp.zeros((48, 4, 128), U32)

                        @pl.when(b == e - 1)
                        def _():
                            for c_ in end_blk(e)[0]:
                                c_.start()

                grow = lambda p: 2 * jnp.maximum(b * U + p - NR, 0)
                for t in range(12 * U):
                    run_slot(t, lambda p: xb.at[slot, p - 3], zero, grow, -99)
                return 0

            if two:
                nost[0] = 1
                lax.fori_loop(0, NR // U, functools.partial(body1), 0)
                nost[0] = 0
            lax.fori_loop(NR // U if two else 0, NB, body1, 0)
            drain(2 * NS - 1 - cut)

        if do1:
            pl.run_scoped(
                pass1,
                pltpu.VMEM((2, XN, 49, 8, 128), U32),
                [pltpu.VMEM((16 // NSB, 2, NT, 8, 128), U32)] * NSB,
                [pltpu.VMEM((1, 8 * C + 16, 128), F32)] * 4,
                pltpu.VMEM((4, C // 2, 512), U32),
                pltpu.VMEM((1, MC, 512), F32),
            )

        def finish_grn():
            ss = jnp.sum(pltpu.bitcast(wb[0, AC:AC + E], F32).T, axis=0, keepdims=True)
            gx = jnp.sqrt(ss * (_GS * _GS) + 1e-6)
            nx = gx / (jnp.sum(gx, axis=1, keepdims=True) * (1.0 / E) + 1e-6)
            gam = gam_ref[...].astype(F32).reshape(1, E)
            bet = bet_ref[...].astype(F32).reshape(1, E)
            w2 = w2t_ref[...].astype(F32)
            w2s = pltpu.bitcast((w2 * ((gam * nx + 1.0) * _GS)).astype(BF16), U32)
            for k in range(3):
                wb[0, W2 + 48 * k:W2 + 48 * k + 48] = w2s[:, 128 * k:128 * k + 128]
            bias[0] = jnp.broadcast_to(jnp.sum(w2 * bet, axis=1, keepdims=True), (C, 128))

        def pass2(xs, xr, tb, cb, zb, gt):
            z16 = zb.bitcast(BF16)
            gt16 = gt.bitcast(BF16)
            RR, SR = 2 * RA, 2 * SA

            def s_in(i, slot):
                return pltpu.make_async_copy(xn_hbm.at[pl.ds(2 * NR + SR * i, SR)], xs.at[slot], sem.at[4 + slot])

            def s_out(i, slot):
                return pltpu.make_async_copy(xs.at[slot], o_hbm.at[pl.ds(2 * NR + SR * i, SR)], sem.at[7 + slot])

            def r_in(i):
                return pltpu.make_async_copy(xn_hbm.at[pl.ds(RR * i, RR)], xr.at[pl.ds(RR * (i & 3), RR)], sem.at[i & 3])

            def r_out(i):
                return pltpu.make_async_copy(xr.at[pl.ds(RR * (i & 3), RR)], o_hbm.at[pl.ds(RR * i, RR)], sem.at[10 + (i & 3)])

            def anchor(v, zero):
                wb[zero, AN:AN + 8] = pltpu.bitcast(v[-8:, -128:], U32)

            prev = []

            def stage_v(g, rows, c_out, zero, lag=lag):
                w = [tb[0, C * t + 8 * g:C * t + 8 * g + 8] for t in range(9)]
                d = [None if r is None else r[8 * g:8 * g + 8, :].astype(F32) for r in rows]
                z = jnp.zeros((8, 128), F32)
                ms, rs = [], []
                for o in range(2):
                    part = [[tree([d[o + i][:, 128 * j:128 * j + 128] * w[3 * i + dx] for i in range(3) if d[o + i] is not None])
                             for j in range(NT)] for dx in range(3)]
                    r = [pltpu.roll(t, 1, 1) for t in part[0]]
                    l = [pltpu.roll(t, 127, 1) for t in part[2]]
                    for j in range(NT):
                        res = (part[1][j] + jnp.where(lane == 0, r[j - 1] if j > 0 else z, r[j])
                               + jnp.where(lane == 127, l[j + 1] if j < NT - 1 else z, l[j]))
                        c_out[(4 * o + j) * C + 8 * g:(4 * o + j) * C + 8 * g + 8] = res
                        rs.append(res)
                    ms += part[1]
                res = tree(rs)
                pin = (tree(ms + prev) if lag == 1 else (prev + [res])[0]) if lag else res
                prev[:] = [res]
                tb[zero, 9 * C:9 * C + 8] = pin
                xr[4 * RR + zero, 0:8, 0:256] = jnp.concatenate([pin, pin], axis=1).astype(BF16)
                return res

            r_in(0).start()
            r_in(1).start()
            s_in(0, 0).start()
            finish_grn()
            for t, v in enumerate(taps()):
                tb[0, C * t:C * t + C] = v
            r_in(0).wait()
            for p in range(2):
                for g in range(NG):
                    stage_v(g, [None if r < 0 else xr.at[r] for r in range(2 * p - 1, 2 * p + 3)], cb.at[p], zs[0], 1)
            for q in range(8):
                stage_b1(q, cb.at[0], 0)
            stage_b2(cb.at[0], 0)
            for q in range(8):
                stage_b3(q, cb.at[0], z16, 0)

            def mm2(rhs, xrow, h, zj):
                o = []
                for j in (2 * h, 2 * h + 1):
                    lhs = jnp.concatenate([wb[zj[j], W2 + 48 * k:W2 + 48 * k + 48] for k in range(3)], axis=1)
                    o.append(jnp.dot(pltpu.bitcast(lhs, BF16), rhs[:, 128 * j:128 * j + 128], preferred_element_type=F32) + bias[zj[j]])

                def fin():
                    res = jnp.concatenate(o, axis=1) + xrow[:, 256 * h:256 * h + 256].astype(F32)
                    xrow[:, 256 * h:256 * h + 256] = res.astype(BF16)
                    return res
                return fin

            def body2(i, s3):
                zero = zs[0]
                zj = [zs[1 + j] for j in range(NT)]
                s3p = jnp.where(s3 == 0, 2, s3 - 1)
                s3n = jnp.where(s3 == 2, 0, s3 + 1)

                NOD = 1000 if nodma else 0

                @pl.when(i >= 1 + NOD)
                def _():
                    s_out(i - 1, s3p).start()
                    r_out(i - 1).start()

                @pl.when(i >= 2 + NOD)
                def _():
                    s_out(i - 2, s3n).wait()
                    r_out(i - 2).wait()

                @pl.when(i < NI - 1 - NOD)
                def _():
                    r_in(i + 2).start()
                    s_in(i + 1, s3n).start()

                @pl.when(i == 0 if nodma else True)
                def _():
                    r_in(i + 1).wait()
                    s_in(i, s3).wait()

                xrow = lambda r: xr.at[RR * ((i + r // RR) & 3) + r % RR]
                prev.clear()
                late = []
                now = [0]

                def flush(n):
                    for d, f in [w for w in late if w[0] <= now[0]]:
                        v = f()
                        if v is not None:
                            anchor(v, zero)
                    late[:] = [w for w in late if w[0] > now[0]]
                    now[0] += n

                ns = 0
                for k in range(RA):
                    e = (i * RA + k) & 1
                    nv = 0
                    for tok in plan[k].split():
                        if tok[0] == "C":
                            o, m, n = (int(ch) for ch in (tok + "06")[1:4])
                            flush(n * MC)
                            zz = mm1(m, z16[o], n)
                            for u in range(n):
                                late.append((now[0] - (n - 1 - u) * MC + DC, lambda m=m, u=u, zz=zz, o=o: act(
                                    m + u, zz[u * MC:(u + 1) * MC], gt16, zero + o * (NGT - 1), None)))
                        elif tok[0] == "S":
                            for h in range(2):
                                flush(96 + 96 * h)
                                late.append((now[0] + 96 * (1 - h) + DD, mm2(G16.at[SR * i + ns], xs.at[s3, ns], h, zj)))
                            ns += 1
                        elif tok[0] == "R":
                            for h in range(2):
                                flush(96 + 96 * h)
                                late.append((now[0] + 96 * (1 - h) + DD, mm2(gt16.at[int(tok[1]) * (NGT - 1)], xrow(2 * k + int(tok[1])), h, zj)))
                        elif tok[0] == "V":
                            for g in range(nv, nv + int(tok[1])):
                                v = stage_v(g, [xrow(r) for r in range(2 * k + 3, 2 * k + 7)], cb.at[e], zero)
                                late.append((now[0] + DV, lambda v=v: v))
                            nv += int(tok[1])
                        elif tok[0] == "B":
                            for q in map(int, tok[1:]):
                                late.append((now[0] + DB, stage_b1(q, cb.at[1 - e], zero, True)))
                        elif tok[0] == "Q":
                            assert not any(f.__name__ == 'put' for _, f in late)
                            late.append((now[0] + DQ, stage_b2(None, zero)))
                        elif tok[0] == "Z":
                            assert not any(f.__name__ == 'put' for _, f in late)
                            for q in map(int, tok[1:]):
                                stage_b3(q, cb.at[1 - e], z16, zero, True)
                    assert nv == NG
                assert ns == SR
                now[0] = 1 << 30
                flush(0)
                return s3n

            lax.fori_loop(0, NI if nodma < 2 else nodma, body2, 0)
            s_out(NI - 1, (NI - 1) % 3).start()
            r_out(NI - 1).start()
            for i in (NI - 2, NI - 1)[min(nodma, 1):]:
                s_out(i, i % 3).wait()
                r_out(i).wait()

        if do2:
            pl.run_scoped(
                pass2,
                pltpu.VMEM((3, 2 * SA, C, 512), BF16),
                pltpu.VMEM((8 * RA + 1, C, 512), BF16),
                pltpu.VMEM((1, 9 * C + 8, 128), F32),
                pltpu.VMEM((2, 8 * C + 16, 128), F32),
                pltpu.VMEM((2, C // 2, 512), U32),
                pltpu.VMEM((NGT, E // 2, 512), U32),
            )
        else:
            def keep(buf):
                buf[...] = G16[zs[0], 0:16]
                pltpu.sync_copy(buf, o_hbm.at[0, pl.ds(0, 16)])
            pl.run_scoped(keep, pltpu.VMEM((16, 512), BF16))

    @jax.jit
    def f(x, dw, w1, w2, grn_gamma, grn_beta):
        xt = x.reshape(512, NT, 128, NG, 8).transpose(0, 3, 1, 4, 2).reshape(NP, 2, NG * NT, 8, 128)
        xn = x.reshape(512, 512, C).transpose(0, 2, 1)
        vm = pl.BlockSpec(memory_space=pltpu.VMEM)
        hb = pl.BlockSpec(memory_space=pl.ANY)
        o = pl.pallas_call(
            kern,
            out_shape=jax.ShapeDtypeStruct(xn.shape, xn.dtype),
            in_specs=[hb, hb, vm, vm, vm, vm, vm],
            out_specs=hb,
            scratch_shapes=[
                pltpu.VMEM((2 * NS - cut, E // 2, 512), U32),
                pltpu.VMEM((1, WB, 128), U32),
                pltpu.VMEM((1, C, 128), F32),
                pltpu.SMEM((1 + NT,), jnp.int32),
                pltpu.SemaphoreType.DMA((14,)),
            ],
            compiler_params=pltpu.CompilerParams(vmem_limit_bytes=128 << 20, flags=flags, disable_bounds_checks=True),
            name="cnx",
        )(xt, xn, dw, w1, w2.T, grn_gamma, grn_beta)
        return o.transpose(0, 2, 1).reshape(x.shape)
    return f


pallas_standalone__modern_conv_block_convnext_v2__vision_kernel = build()
```

```python
import math

import jax
import jax.numpy as jnp
from jax import lax
import jax.experimental.pallas as pl
import jax.experimental.pallas.tpu as pltpu

F32, BF16, U32 = jnp.float32, jnp.bfloat16, jnp.uint32
H, W, C, E = 512, 512, 96, 384
NG, NT = C // 8, W // 128
NP = H // 2
MC = 64
NM = E // MC

_C0 = math.sqrt(2.0 / math.pi)
_K = (_C0 * 0.044715) ** (1.0 / 3.0)
_B = _C0 / _K
_GS = 0.5 / _K

U = 8
NB = NP // U
XN = U + 2
SR, RR = 10, 6
NI = H // (SR + RR)
NR = RR * NI // 2

W1, S1, S2, AN, AW, AC = 0, 192, 264, 336, 352, 448
W2, WB = AW, AC + E
CR, CP, CB = 8 * C, 8 * C + 8, 8 * C + 32
TP, TR, TB = 9 * C, 9 * C + 32, 9 * C + 96


def _tree(v):
    while len(v) > 1:
        v = [v[i] + v[i + 1] if i + 1 < len(v) else v[i] for i in range(0, len(v), 2)]
    return v[0]


def _shift(prv, nxt):
    lane = lax.broadcasted_iota(jnp.int32, (8, 128), 1)
    zero = jnp.zeros_like(prv[0])
    r = [zero] + [pltpu.roll(t, 1, 1) for t in prv]
    l = [pltpu.roll(t, 127, 1) for t in nxt] + [zero]
    return ([jnp.where(lane == 0, r[j], r[j + 1]) for j in range(NT)],
            [jnp.where(lane == 127, l[j + 1], l[j]) for j in range(NT)])


def _gelu(z):
    return z + z * jnp.tanh(z * (z * z + _B))


def _kernel(xt_hbm, x_hbm, dw_ref, w1_ref, w2t_ref, gam_ref, bet_ref, o_hbm, kept, rstd, wb, zs, sem):
    x32 = xt_hbm.bitcast(U32)
    kept16 = kept.bitcast(BF16)
    for j in range(NT):
        zs[j] = 0

    def taps():
        d = dw_ref[...].astype(F32)
        m = jnp.concatenate([d[i, j:j + 1, :] for i in range(3) for j in range(3)] + [jnp.zeros((128 - 9, C), F32)], axis=0)
        m = jnp.concatenate([m, jnp.zeros((128, 128 - C), F32)], axis=1).T[:C]
        return [jnp.broadcast_to(m[:, t:t + 1], (C, 128)) for t in range(9)]

    def mm1(m, n, z):
        lhs = pltpu.bitcast(wb[0, W1 + m * MC // 2:W1 + (m + n) * MC // 2], BF16)[:, :C]
        return jnp.dot(lhs, z, preferred_element_type=F32)

    def put_act(dst, row, m, g):
        dst[pl.ds(row, 1), m * MC:(m + 1) * MC, :] = g[None].astype(BF16)

    def anchor(v, zero):
        wb[zero, AN:AN + 8] = pltpu.bitcast(v[-8:, -128:], U32)

    def pass1(xb, sbs, cbs, zb, raw):
        z16 = zb.bitcast(BF16)

        def load(slot, p_hi, n_hi, off_hi, p_lo, n_lo):
            return [
                pltpu.make_async_copy(x32.at[pl.ds(p_hi - 1, n_hi), 1],
                                      xb.at[slot, pl.ds(off_hi, n_hi), pl.ds(0, 48), pl.ds(0, 4)], sem.at[slot]),
                pltpu.make_async_copy(x32.at[pl.ds(p_lo, n_lo), 0],
                                      xb.at[slot, pl.ds(0, n_lo), pl.ds(0, 48), pl.ds(4, 4)], sem.at[2 + slot]),
            ]

        def block(b, slot):
            return load(slot, b * U + 3, XN, 0, b * U + 3, XN)

        def last_block():
            return load((NB - 1) & 1, NP - U + 3, U - 2, 0, NP - U + 3, U - 3)

        def prep_weights():
            tp = taps()
            r = lax.broadcasted_iota(jnp.int32, (C, 128), 0)
            k = lax.broadcasted_iota(jnp.int32, (C, 128), 1)
            key = jnp.where((r & 7) == (k & 7), k >> 3, -1)
            mats = []
            for o in range(2):
                a = jnp.zeros((C, 128), F32)
                for i in range(3):
                    for j in range(3):
                        a = jnp.where(key == ((i + o) // 2 * 3 + j) * 2 + (i + o) % 2, tp[3 * i + j], a)
                mats.append(a)
            for g in range(NG):
                a = jnp.concatenate([t[8 * g:8 * g + 8] for t in mats], axis=0)
                wb[0, AW + 8 * g:AW + 8 * g + 8] = pltpu.bitcast(a.astype(BF16), U32)
            w = w1_ref[...].astype(F32)
            w = w - jnp.sum(w, axis=0, keepdims=True) * (1.0 / C)
            w = jnp.concatenate([w, jnp.zeros((128 - C, E), F32)], axis=0)
            wb[0, W1:W1 + E // 2] = pltpu.bitcast(w.T.astype(BF16), U32)
            wb[0, AC:AC + E] = jnp.zeros((E, 128), U32)
            raw[...] = jnp.zeros_like(raw)

        def shift(src, g, dst, zero):
            v = [src[NT * g + j] for j in range(NT)]
            for d, part in enumerate(_shift(v, v)):
                for j in range(NT):
                    dst[zero, d, j] = part[j]

        def conv(g, halves, cb, zero):
            cols = [jnp.concatenate([t for src, sb in halves for t in (sb[0, 0, j], src[NT * g + j], sb[0, 1, j])], axis=0)
                    for j in range(NT)]
            res = jnp.dot(pltpu.bitcast(wb[0, AW + 8 * g:AW + 8 * g + 8], BF16)[:, :C],
                          pltpu.bitcast(jnp.concatenate(cols, axis=1), BF16), preferred_element_type=F32)
            for q in range(2 * NT):
                o, j = divmod(q, NT)
                cb[zero, q * C + 8 * g:q * C + 8 * g + 8] = res[8 * o:8 * o + 8, 128 * j:128 * j + 128]

        def ln_sums(q, cb, zero):
            c = [cb[0, q * C + 8 * g:q * C + 8 * g + 8] for g in range(NG)]
            s1, s2 = c[0], c[0] * c[0]
            for t in c[1:]:
                s1, s2 = s1 + t, s2 + t * t
            wb[zero, S1 + 9 * q:S1 + 9 * q + 8] = pltpu.bitcast(s1, U32)
            wb[zero, S2 + 9 * q:S2 + 9 * q + 8] = pltpu.bitcast(s2, U32)

        def ln_rstd(cb, pair, zero):
            s1, s2 = (_tree([pltpu.bitcast(wb[0, pl.ds(s + i, 8, stride=9), :], F32) for i in range(8)]) for s in (S1, S2))
            var = jnp.maximum(s2 - s1 * s1 * (1.0 / C), 0.0)
            r = lax.rsqrt(var * (1.0 / (C * _K * _K)) + 1e-5 / (_K * _K))
            cb[zero, CR:CR + 8] = r
            rstd[jnp.minimum(pair, NR)] = r
            return r

        def ln_scale(q, cb, zrow):
            o, j = divmod(q, NT)
            z = cb[0, q * C:(q + 1) * C] * cb[0, CR + q:CR + q + 1]
            z16[pl.ds(zrow + o, 1), :, 128 * j:128 * j + 128] = z[None].astype(BF16)

        def act(m, z, row, zero):
            g = _gelu(z)
            put_act(kept16, row, m, g)
            sq = g * g
            rows = slice(AC + m * MC, AC + (m + 1) * MC)
            tot = pltpu.bitcast(wb[0, rows], F32) + _tree([sq[:, 128 * j:128 * j + 128] for j in range(NT)])
            wb[zero, rows] = pltpu.bitcast(tot, U32)

        def run(slots, xp, p0, first):
            zero = zs[0]
            hid = {}
            live = (lambda p: p >= 0) if first else (lambda p: True)

            def finish(t):
                p, q = divmod(t, 12)
                row = 2 * jnp.maximum(p0 + p - NR, 0) + q // NM
                act(q % NM, raw[...] if t < 0 else hid[t], row, zero)

            for t in slots:
                p, q = divmod(t, 12)
                if t - 2 in hid:
                    pin = hid[t - 2][0:8, 0:128]
                    xb[zero, 0, 48] = pltpu.bitcast(pin, U32)
                    if q >= 8:
                        cbs[(p + 1) & 3][zero, CP:CP + 8] = pin
                n = t + 53
                if live(n // 12):
                    shift(xp(n // 12), n % 12, sbs[n & 15], zero)
                if not first:
                    hid[t] = mm1(q % NM, 1, z16[2 * (p & 1) + q // NM])
                    if t == slots[-1]:
                        raw[...] = hid[t]
                if live(p + 2):
                    if q < 8:
                        ln_sums(q, cbs[(p + 2) & 3], zero)
                    elif q == 8:
                        r = ln_rstd(cbs[(p + 2) & 3], p0 + p + 2, zero)
                    elif q == 9:
                        anchor(r, zero)
                if live(p + 1) and q >= 8:
                    for k in (2 * q - 16, 2 * q - 15):
                        ln_scale(k, cbs[(p + 1) & 3], 2 * ((p + 1) & 1) + zero)
                n = t + 38
                if live(n // 12):
                    conv(n % 12, [(xp(n // 12 + k), sbs[(n + 12 * k) & 15]) for k in range(2)], cbs[(n // 12) & 3], zero)
                if not first:
                    for tf in [-1] if t == 0 else range(max(t - 2, 0), t if t == slots[-1] else t - 1):
                        finish(tf)

        head = load(1, 1, 4, 1, 0, 5)
        for cp in head + block(0, 0):
            cp.start()
        prep_weights()
        for cp in head:
            cp.wait()
        xb[1, 0, 0:48, 0:4, :] = jnp.zeros((48, 4, 128), U32)
        run(range(-53, 0), lambda p: xb.at[1, p], 0, True)

        def body(b, carry):
            slot = b & 1

            @pl.when(b < NB - 1)
            def _():
                for cp in block(b, slot):
                    cp.wait()

            @pl.when(b < NB - 2)
            def _():
                for cp in block(b + 1, 1 - slot):
                    cp.start()

            @pl.when(b >= NB - 2)
            def _():
                @pl.when(b == NB - 1)
                def _():
                    for cp in last_block():
                        cp.wait()
                    xb[(NB - 1) & 1, U - 3, 0:48, 4:8, :] = jnp.zeros((48, 4, 128), U32)

                @pl.when(b == NB - 2)
                def _():
                    for cp in last_block():
                        cp.start()

            run(range(12 * U), lambda p: xb.at[slot, p - 3], b * U, False)
            return carry

        lax.fori_loop(0, NB, body, 0)
        act(NM - 1, raw[...], SR * NI - 1, 0)

    pl.run_scoped(
        pass1,
        pltpu.VMEM((2, XN, 50, 8, 128), U32),
        [pltpu.VMEM((1, 2, NT, 8, 128), U32)] * 16,
        [pltpu.VMEM((1, CB, 128), F32)] * 4,
        pltpu.VMEM((4, C // 2, W), U32),
        pltpu.VMEM((MC, W), F32),
    )

    def pass2(xs, xr, tb, bias, zbs, gt):
        gt16 = gt.bitcast(BF16)

        def s_in(i, slot):
            return pltpu.make_async_copy(x_hbm.at[pl.ds(2 * NR + SR * i, SR)], xs.at[slot], sem.at[4 + slot])

        def s_out(i, slot):
            return pltpu.make_async_copy(xs.at[slot], o_hbm.at[pl.ds(2 * NR + SR * i, SR)], sem.at[7 + slot])

        def r_in(i):
            return pltpu.make_async_copy(x_hbm.at[pl.ds(RR * i, RR)], xr.at[pl.ds(RR * (i & 3), RR)], sem.at[i & 3])

        def r_out(i):
            return pltpu.make_async_copy(xr.at[pl.ds(RR * (i & 3), RR)], o_hbm.at[pl.ds(RR * i, RR)], sem.at[10 + (i & 3)])

        def prep_weights():
            ss = jnp.sum(pltpu.bitcast(wb[0, AC:AC + E], F32).T, axis=0, keepdims=True)
            gx = jnp.sqrt(ss * (_GS * _GS) + 1e-6)
            nx = gx / (jnp.sum(gx, axis=1, keepdims=True) * (1.0 / E) + 1e-6)
            gamma = gam_ref[...].astype(F32).reshape(1, E)
            beta = bet_ref[...].astype(F32).reshape(1, E)
            w2 = w2t_ref[...].astype(F32)
            w2s = pltpu.bitcast((w2 * ((gamma * nx + 1.0) * _GS)).astype(BF16), U32)
            for k in range(E // 128):
                wb[0, W2 + 48 * k:W2 + 48 * k + 48] = w2s[:, 128 * k:128 * k + 128]
            bias[0] = jnp.broadcast_to(jnp.sum(w2 * beta, axis=1, keepdims=True), (C, 128))
            for t, v in enumerate(taps()):
                tb[0, C * t:C * t + C] = v

        def conv_ln(g, rows, pair, zb, zero, before=None):
            if g == 0:
                for q in range(2 * NT):
                    tb[zero, TR + 8 * q:TR + 8 * q + 8] = jnp.broadcast_to(rstd[pair, q:q + 1], (8, 128))
            w = [tb[0, C * t + 8 * g:C * t + 8 * g + 8] for t in range(9)]
            d = [None if r is None else r[8 * g:8 * g + 8, :].astype(F32) for r in rows]
            mids, outs = [], []
            for o in range(2):
                part = [[_tree([d[o + i][:, 128 * j:128 * j + 128] * w[3 * i + dx] for i in range(3) if d[o + i] is not None])
                         for j in range(NT)] for dx in range(3)]
                c = [m + a + b for m, a, b in zip(part[1], *_shift(part[0], part[2]))]
                z = [c[j] * tb[0, TR + 8 * (NT * o + j):TR + 8 * (NT * o + j) + 8] for j in range(NT)]
                zb[zero, o, 8 * g:8 * g + 8, :] = jnp.concatenate(z, axis=1).astype(BF16)
                mids += part[1]
                outs += c
            done = _tree(outs)
            pin = done if before is None else _tree(mids + before)
            tb[zero, TP:TP + 8] = pin
            xr[4 * RR + zero, 0:8, 0:256] = jnp.concatenate([pin, pin], axis=1).astype(BF16)
            return done

        def mm2(g, xrow, half, zj):
            lhs = pltpu.bitcast(jnp.concatenate([wb[0, W2 + 48 * k:W2 + 48 * k + 48] for k in range(E // 128)], axis=1), BF16)
            o = [jnp.dot(lhs, g[:, 128 * j:128 * j + 128], preferred_element_type=F32) + bias[zj[j]]
                 for j in (2 * half, 2 * half + 1)]

            def finish():
                res = jnp.concatenate(o, axis=1) + xrow[:, 256 * half:256 * half + 256].astype(F32)
                xrow[:, 256 * half:256 * half + 256] = res.astype(BF16)
                return res
            return finish

        r_in(0).start()
        r_in(1).start()
        s_in(0, 0).start()
        prep_weights()
        r_in(0).wait()
        before = []
        for p in range(2):
            for g in range(NG):
                rows = [None if r < 0 else xr.at[r] for r in range(2 * p - 1, 2 * p + 3)]
                before = [conv_ln(g, rows, p, zbs[p], zs[0], before)]

        def body(i, cur):
            zj = [zs[j] for j in range(NT)]
            zero = zj[0]
            prv = jnp.where(cur == 0, 2, cur - 1)
            nxt = jnp.where(cur == 2, 0, cur + 1)

            @pl.when(i >= 1)
            def _():
                s_out(i - 1, prv).start()
                r_out(i - 1).start()

            @pl.when(i >= 2)
            def _():
                s_out(i - 2, nxt).wait()
                r_out(i - 2).wait()

            @pl.when(i < NI - 1)
            def _():
                r_in(i + 2).start()
                s_in(i + 1, nxt).start()

            r_in(i + 1).wait()
            s_in(i, cur).wait()

            def xrow(r):
                return xr.at[RR * ((i + r // RR) & 3) + r % RR]

            late = []
            now = [0]

            def advance(cycles):
                for deadline, work in late:
                    if deadline <= now[0]:
                        anchor(work(), zero)
                late[:] = [w for w in late if w[0] > now[0]]
                now[0] += cycles

            def hidden(z):
                advance(E)
                h = mm1(0, NM, z[...])

                def finish(m):
                    g = _gelu(h[m * MC:(m + 1) * MC])
                    put_act(gt16, zero, m, g)
                    return g
                late.extend((now[0] - (NM - 1 - m) * MC + 160, lambda m=m: finish(m)) for m in range(NM))

            def output(g, row):
                for half in range(2):
                    advance(C * (1 + half))
                    late.append((now[0] + C * (1 - half) + 150, mm2(g, row, half, zj)))

            ns = 0
            for k in range(RR // 2):
                ng = 0
                for op in "0v svv avv 1v svv bvv svv" + (" s" if k == 2 else ""):
                    if op in "01":
                        hidden(zbs[k].at[0, int(op)])
                    elif op in "ab":
                        output(gt16.at[0], xrow(2 * k + "ab".index(op)))
                    elif op == "s":
                        output(kept16.at[SR * i + ns], xs.at[cur, ns])
                        ns += 1
                    elif op == "v":
                        v = conv_ln(ng, [xrow(r) for r in range(2 * k + 3, 2 * k + 7)],
                                    jnp.minimum(RR // 2 * i + k + 2, NR), zbs[(k + 2) % 3], zero)
                        late.append((now[0] + 500, lambda v=v: v))
                        ng += 1
            now[0] += 1000
            advance(0)
            return nxt

        lax.fori_loop(0, NI, body, 0)
        s_out(NI - 1, (NI - 1) % 3).start()
        r_out(NI - 1).start()
        for i in (NI - 2, NI - 1):
            s_out(i, i % 3).wait()
            r_out(i).wait()

    pl.run_scoped(
        pass2,
        pltpu.VMEM((3, SR, C, W), BF16),
        pltpu.VMEM((4 * RR + 1, C, W), BF16),
        pltpu.VMEM((1, TB, 128), F32),
        pltpu.VMEM((1, C, 128), F32),
        [pltpu.VMEM((1, 2, C, W), BF16)] * 3,
        pltpu.VMEM((1, E // 2, W), U32),
    )


@jax.jit
def pallas_standalone__modern_conv_block_convnext_v2__vision_kernel(
    x: jax.Array,
    dw: jax.Array,
    w1: jax.Array,
    w2: jax.Array,
    grn_gamma: jax.Array,
    grn_beta: jax.Array,
):
    tiles = x.reshape(H, NT, 128, NG, 8).transpose(0, 3, 1, 4, 2).reshape(NP, 2, NG * NT, 8, 128)
    rows = x.reshape(H, W, C).transpose(0, 2, 1)
    vmem = pl.BlockSpec(memory_space=pltpu.VMEM)
    hbm = pl.BlockSpec(memory_space=pl.ANY)
    out = pl.pallas_call(
        _kernel,
        out_shape=jax.ShapeDtypeStruct(rows.shape, rows.dtype),
        in_specs=[hbm, hbm, vmem, vmem, vmem, vmem, vmem],
        out_specs=hbm,
        scratch_shapes=[
            pltpu.VMEM((SR * NI, E // 2, W), U32),
            pltpu.VMEM((NR + 1, 8, 128), F32),
            pltpu.VMEM((1, WB, 128), U32),
            pltpu.SMEM((NT,), jnp.int32),
            pltpu.SemaphoreType.DMA((14,)),
        ],
        compiler_params=pltpu.CompilerParams(vmem_limit_bytes=128 << 20, disable_bounds_checks=True),
        name="cnx",
    )(tiles, rows, dw, w1, w2.T, grn_gamma, grn_beta)
    return out.transpose(0, 2, 1).reshape(x.shape)
```

```python
import math

import jax
import jax.numpy as jnp
from jax import lax
import jax.experimental.pallas as pl
import jax.experimental.pallas.tpu as pltpu

F32, BF16, U32 = jnp.float32, jnp.bfloat16, jnp.uint32
H, W, C, E = 512, 512, 96, 384
NG, NT = C // 8, W // 128
NP = H // 2
MC = 64
NM = E // MC

_C0 = math.sqrt(2.0 / math.pi)
_K = (_C0 * 0.044715) ** (1.0 / 3.0)
_B = _C0 / _K
_GS = 0.5 / _K

U = 8
SUMS, SCALE = (0, 1, 2, 3, 4, 5, 6, 7), (4, 5, 6, 7, 8, 9, 10, 11)
NB = NP // U
XN = U + 2
SR, RR = 10, 6
NI = H // (SR + RR)
NR = RR * NI // 2

W1, S1, S2, AN, AW, AC = 0, 192, 264, 336, 352, 448
W2, WB = AW, AC + E
CR, CP, CB = 8 * C, 8 * C + 8, 8 * C + 32
TP, TR, TB = 9 * C, 9 * C + 32, 9 * C + 96


def _tree(v):
    while len(v) > 1:
        v = [v[i] + v[i + 1] if i + 1 < len(v) else v[i] for i in range(0, len(v), 2)]
    return v[0]


def _shift(prv, nxt):
    lane = lax.broadcasted_iota(jnp.int32, (8, 128), 1)
    zero = jnp.zeros_like(prv[0])
    r = [zero] + [pltpu.roll(t, 1, 1) for t in prv]
    l = [pltpu.roll(t, 127, 1) for t in nxt] + [zero]
    return ([jnp.where(lane == 0, r[j], r[j + 1]) for j in range(NT)],
            [jnp.where(lane == 127, l[j + 1], l[j]) for j in range(NT)])


def _gelu(z):
    return z + z * jnp.tanh(z * (z * z + _B))


def _kernel(xt_hbm, x_hbm, dw_ref, w1_ref, w2t_ref, gam_ref, bet_ref, o_hbm, kept, rstd, wb, zs, sem):
    x32 = xt_hbm.bitcast(U32)
    kept16 = kept.bitcast(BF16)
    for j in range(NT):
        zs[j] = 0

    def taps():
        d = dw_ref[...].astype(F32)
        m = jnp.concatenate([d[i, j:j + 1, :] for i in range(3) for j in range(3)] + [jnp.zeros((128 - 9, C), F32)], axis=0)
        m = jnp.concatenate([m, jnp.zeros((128, 128 - C), F32)], axis=1).T[:C]
        return [jnp.broadcast_to(m[:, t:t + 1], (C, 128)) for t in range(9)]

    def mm1(m, n, z):
        lhs = pltpu.bitcast(wb[0, W1 + m * MC // 2:W1 + (m + n) * MC // 2], BF16)[:, :C]
        return jnp.dot(lhs, z, preferred_element_type=F32)

    def put_act(dst, row, m, g):
        dst[pl.ds(row, 1), m * MC:(m + 1) * MC, :] = g[None].astype(BF16)

    def anchor(v, zero):
        wb[zero, AN:AN + 8] = pltpu.bitcast(v[-8:, -128:], U32)

    def pass1(xb, sbs, cbs, zb, raw):
        z16 = zb.bitcast(BF16)

        def load(slot, p_hi, n_hi, off_hi, p_lo, n_lo):
            return [
                pltpu.make_async_copy(x32.at[pl.ds(p_hi - 1, n_hi), 1],
                                      xb.at[slot, pl.ds(off_hi, n_hi), pl.ds(0, 48), pl.ds(0, 4)], sem.at[slot]),
                pltpu.make_async_copy(x32.at[pl.ds(p_lo, n_lo), 0],
                                      xb.at[slot, pl.ds(0, n_lo), pl.ds(0, 48), pl.ds(4, 4)], sem.at[2 + slot]),
            ]

        def block(b, slot):
            return load(slot, b * U + 3, XN, 0, b * U + 3, XN)

        def last_block():
            return load((NB - 1) & 1, NP - U + 3, U - 2, 0, NP - U + 3, U - 3)

        def prep_weights():
            tp = taps()
            r = lax.broadcasted_iota(jnp.int32, (C, 128), 0)
            k = lax.broadcasted_iota(jnp.int32, (C, 128), 1)
            key = jnp.where((r & 7) == (k & 7), k >> 3, -1)
            mats = []
            for o in range(2):
                a = jnp.zeros((C, 128), F32)
                for i in range(3):
                    for j in range(3):
                        a = jnp.where(key == ((i + o) // 2 * 3 + j) * 2 + (i + o) % 2, tp[3 * i + j], a)
                mats.append(a)
            for g in range(NG):
                a = jnp.concatenate([t[8 * g:8 * g + 8] for t in mats], axis=0)
                wb[0, AW + 8 * g:AW + 8 * g + 8] = pltpu.bitcast(a.astype(BF16), U32)
            w = w1_ref[...].astype(F32)
            w = w - jnp.sum(w, axis=0, keepdims=True) * (1.0 / C)
            w = jnp.concatenate([w, jnp.zeros((128 - C, E), F32)], axis=0)
            wb[0, W1:W1 + E // 2] = pltpu.bitcast(w.T.astype(BF16), U32)
            wb[0, AC:AC + E] = jnp.zeros((E, 128), U32)
            raw[...] = jnp.zeros_like(raw)

        def shift(src, g, dst, zero):
            v = [src[NT * g + j] for j in range(NT)]
            for d, part in enumerate(_shift(v, v)):
                for j in range(NT):
                    dst[zero, d, j] = part[j]

        def conv(g, halves, cb, zero):
            cols = [jnp.concatenate([t for src, sb in halves for t in (sb[0, 0, j], src[NT * g + j], sb[0, 1, j])], axis=0)
                    for j in range(NT)]
            res = jnp.dot(pltpu.bitcast(wb[0, AW + 8 * g:AW + 8 * g + 8], BF16)[:, :C],
                          pltpu.bitcast(jnp.concatenate(cols, axis=1), BF16), preferred_element_type=F32)
            for q in range(2 * NT):
                o, j = divmod(q, NT)
                cb[zero, q * C + 8 * g:q * C + 8 * g + 8] = res[8 * o:8 * o + 8, 128 * j:128 * j + 128]

        def ln_sums(q, cb, zero):
            c = [cb[0, q * C + 8 * g:q * C + 8 * g + 8] for g in range(NG)]
            s1, s2 = c[0], c[0] * c[0]
            for t in c[1:]:
                s1, s2 = s1 + t, s2 + t * t
            wb[zero, S1 + 9 * q:S1 + 9 * q + 8] = pltpu.bitcast(s1, U32)
            wb[zero, S2 + 9 * q:S2 + 9 * q + 8] = pltpu.bitcast(s2, U32)

        def ln_rstd(cb, pair, zero):
            s1, s2 = (_tree([pltpu.bitcast(wb[0, pl.ds(s + i, 8, stride=9), :], F32) for i in range(8)]) for s in (S1, S2))
            var = jnp.maximum(s2 - s1 * s1 * (1.0 / C), 0.0)
            r = lax.rsqrt(var * (1.0 / (C * _K * _K)) + 1e-5 / (_K * _K))
            cb[zero, CR:CR + 8] = r
            if pair is not None:
                rstd[jnp.minimum(pair, NR)] = r
            return r

        def ln_scale(q, cb, zrow):
            o, j = divmod(q, NT)
            z = cb[0, q * C:(q + 1) * C] * cb[0, CR + q:CR + q + 1]
            z16[pl.ds(zrow + o, 1), :, 128 * j:128 * j + 128] = z[None].astype(BF16)

        def act(m, z, row, zero):
            g = _gelu(z)
            if row is not None:
                put_act(kept16, row, m, g)
            sq = g * g
            rows = slice(AC + m * MC, AC + (m + 1) * MC)
            tot = pltpu.bitcast(wb[0, rows], F32) + _tree([sq[:, 128 * j:128 * j + 128] for j in range(NT)])
            wb[zero, rows] = pltpu.bitcast(tot, U32)

        def run(slots, xp, p0, first, keep):
            zero = zs[0]
            hid = {}
            live = (lambda p: p >= 0) if first else (lambda p: True)

            def finish(t):
                p, q = divmod(t, 12)
                row = 2 * jnp.maximum(p0 + p - NR, 0) + q // NM if keep else None
                act(q % NM, raw[...] if t < 0 else hid[t], row, zero)

            for t in slots:
                p, q = divmod(t, 12)
                if t - 2 in hid:
                    pin = hid[t - 2][0:8, 0:128]
                    xb[zero, 0, 48] = pltpu.bitcast(pin, U32)
                    if q in SCALE:
                        cbs[(p + 1) & 3][zero, CP:CP + 8] = pin
                n = t + 53
                if live(n // 12):
                    shift(xp(n // 12), n % 12, sbs[n & 15], zero)
                if not first:
                    hid[t] = mm1(q % NM, 1, z16[2 * (p & 1) + q // NM])
                    if t == slots[-1]:
                        raw[...] = hid[t]
                if live(p + 2):
                    if q in SUMS:
                        ln_sums(SUMS.index(q), cbs[(p + 2) & 3], zero)
                    elif q == SUMS[-1] + 1:
                        r = ln_rstd(cbs[(p + 2) & 3], None if keep else p0 + p + 2, zero)
                    elif q == SUMS[-1] + 2:
                        anchor(r, zero)
                for k in range(2 * NT):
                    if live(p + 1) and q == SCALE[k]:
                        ln_scale(k, cbs[(p + 1) & 3], 2 * ((p + 1) & 1) + zero)
                n = t + 38
                if live(n // 12):
                    conv(n % 12, [(xp(n // 12 + k), sbs[(n + 12 * k) & 15]) for k in range(2)], cbs[(n // 12) & 3], zero)
                if not first:
                    for tf in [-1] if t == 0 else range(max(t - 2, 0), t if t == slots[-1] else t - 1):
                        finish(tf)

        head = load(1, 1, 4, 1, 0, 5)
        for cp in head + block(0, 0):
            cp.start()
        prep_weights()
        for cp in head:
            cp.wait()
        xb[1, 0, 0:48, 0:4, :] = jnp.zeros((48, 4, 128), U32)
        run(range(-53, 0), lambda p: xb.at[1, p], 0, True, False)

        def body_dropped(b, carry):
            slot = b & 1
            for cp in block(b, slot):
                cp.wait()
            for cp in block(b + 1, 1 - slot):
                cp.start()
            run(range(12 * U), lambda p: xb.at[slot, p - 3], b * U, False, False)
            return carry

        def body_kept(b, carry):
            slot = b & 1

            @pl.when(b < NB - 1)
            def _():
                for cp in block(b, slot):
                    cp.wait()

            @pl.when(b < NB - 2)
            def _():
                for cp in block(b + 1, 1 - slot):
                    cp.start()

            @pl.when(b >= NB - 2)
            def _():
                @pl.when(b == NB - 1)
                def _():
                    for cp in last_block():
                        cp.wait()
                    xb[(NB - 1) & 1, U - 3, 0:48, 4:8, :] = jnp.zeros((48, 4, 128), U32)

                @pl.when(b == NB - 2)
                def _():
                    for cp in last_block():
                        cp.start()

            run(range(12 * U), lambda p: xb.at[slot, p - 3], b * U, False, True)
            return carry

        lax.fori_loop(0, NR // U, body_dropped, 0)
        lax.fori_loop(NR // U, NB, body_kept, 0)
        act(NM - 1, raw[...], SR * NI - 1, 0)

    pl.run_scoped(
        pass1,
        pltpu.VMEM((2, XN, 50, 8, 128), U32),
        [pltpu.VMEM((1, 2, NT, 8, 128), U32)] * 16,
        [pltpu.VMEM((1, CB, 128), F32)] * 4,
        pltpu.VMEM((4, C // 2, W), U32),
        pltpu.VMEM((MC, W), F32),
    )

    def pass2(xs, xr, tb, bias, zbs, gt):
        gt16 = gt.bitcast(BF16)

        def s_in(i, slot):
            return pltpu.make_async_copy(x_hbm.at[pl.ds(2 * NR + SR * i, SR)], xs.at[slot], sem.at[4 + slot])

        def s_out(i, slot):
            return pltpu.make_async_copy(xs.at[slot], o_hbm.at[pl.ds(2 * NR + SR * i, SR)], sem.at[7 + slot])

        def r_in(i):
            return pltpu.make_async_copy(x_hbm.at[pl.ds(RR * i, RR)], xr.at[pl.ds(RR * (i & 3), RR)], sem.at[i & 3])

        def r_out(i):
            return pltpu.make_async_copy(xr.at[pl.ds(RR * (i & 3), RR)], o_hbm.at[pl.ds(RR * i, RR)], sem.at[10 + (i & 3)])

        def prep_weights():
            ss = jnp.sum(pltpu.bitcast(wb[0, AC:AC + E], F32).T, axis=0, keepdims=True)
            gx = jnp.sqrt(ss * (_GS * _GS) + 1e-6)
            nx = gx / (jnp.sum(gx, axis=1, keepdims=True) * (1.0 / E) + 1e-6)
            gamma = gam_ref[...].astype(F32).reshape(1, E)
            beta = bet_ref[...].astype(F32).reshape(1, E)
            w2 = w2t_ref[...].astype(F32)
            w2s = pltpu.bitcast((w2 * ((gamma * nx + 1.0) * _GS)).astype(BF16), U32)
            for k in range(E // 128):
                wb[0, W2 + 48 * k:W2 + 48 * k + 48] = w2s[:, 128 * k:128 * k + 128]
            bias[0] = jnp.broadcast_to(jnp.sum(w2 * beta, axis=1, keepdims=True), (C, 128))
            for t, v in enumerate(taps()):
                tb[0, C * t:C * t + C] = v

        def conv_ln(g, rows, pair, zb, zero, before=None):
            if g == 0:
                for q in range(2 * NT):
                    tb[zero, TR + 8 * q:TR + 8 * q + 8] = jnp.broadcast_to(rstd[pair, q:q + 1], (8, 128))
            w = [tb[0, C * t + 8 * g:C * t + 8 * g + 8] for t in range(9)]
            d = [None if r is None else r[8 * g:8 * g + 8, :].astype(F32) for r in rows]
            mids, outs = [], []
            for o in range(2):
                part = [[_tree([d[o + i][:, 128 * j:128 * j + 128] * w[3 * i + dx] for i in range(3) if d[o + i] is not None])
                         for j in range(NT)] for dx in range(3)]
                c = [m + a + b for m, a, b in zip(part[1], *_shift(part[0], part[2]))]
                z = [c[j] * tb[0, TR + 8 * (NT * o + j):TR + 8 * (NT * o + j) + 8] for j in range(NT)]
                zb[zero, o, 8 * g:8 * g + 8, :] = jnp.concatenate(z, axis=1).astype(BF16)
                mids += part[1]
                outs += c
            done = outs[7] if before is None else _tree(outs)
            pin = done if before is None else _tree(mids + before)
            if before is None:
                for n in range(4):
                    tb[zero, TP + 8 * n:TP + 8 * n + 8] = outs[2 * n] + outs[2 * n + 1]
            else:
                tb[zero, TP:TP + 8] = pin
            xr[4 * RR + zero, 0:8, 0:256] = jnp.concatenate([mids[3], mids[7]] if before is None else [pin, pin], axis=1).astype(BF16)
            return done

        def mm2(g, xrow, half, zj):
            lhs = pltpu.bitcast(jnp.concatenate([wb[0, W2 + 48 * k:W2 + 48 * k + 48] for k in range(E // 128)], axis=1), BF16)
            o = [jnp.dot(lhs, g[:, 128 * j:128 * j + 128], preferred_element_type=F32) + bias[zj[j]]
                 for j in (2 * half, 2 * half + 1)]

            def finish():
                res = jnp.concatenate(o, axis=1) + xrow[:, 256 * half:256 * half + 256].astype(F32)
                xrow[:, 256 * half:256 * half + 256] = res.astype(BF16)
                return res
            return finish

        r_in(0).start()
        r_in(1).start()
        s_in(0, 0).start()
        prep_weights()
        r_in(0).wait()
        before = []
        for p in range(2):
            for g in range(NG):
                rows = [None if r < 0 else xr.at[r] for r in range(2 * p - 1, 2 * p + 3)]
                before = [conv_ln(g, rows, p, zbs[p], zs[0], before)]

        def body(i, cur):
            zj = [zs[j] for j in range(NT)]
            zero = zj[0]
            prv = jnp.where(cur == 0, 2, cur - 1)
            nxt = jnp.where(cur == 2, 0, cur + 1)

            @pl.when(i >= 2)
            def _():
                s_out(i - 2, nxt).wait()
                r_out(i - 2).wait()

            @pl.when(i < NI - 1)
            def _():
                r_in(i + 2).start()
                s_in(i + 1, nxt).start()

            @pl.when(i >= 1)
            def _():
                s_out(i - 1, prv).start()
                r_out(i - 1).start()

            r_in(i + 1).wait()
            s_in(i, cur).wait()

            def xrow(r):
                return xr.at[RR * ((i + r // RR) & 3) + r % RR]

            late = []
            now = [0]

            def advance(cycles):
                for deadline, work in late:
                    if deadline <= now[0]:
                        anchor(work(), zero)
                late[:] = [w for w in late if w[0] > now[0]]
                now[0] += cycles

            def hidden(z):
                advance(E)
                h = mm1(0, NM, z[...])

                def finish(m):
                    g = _gelu(h[m * MC:(m + 1) * MC])
                    put_act(gt16, zero, m, g)
                    return g
                late.extend((now[0] - (NM - 1 - m) * MC + 160, lambda m=m: finish(m)) for m in range(NM))

            def output(g, row):
                for half in range(2):
                    advance(C * (1 + half))
                    late.append((now[0] + C * (1 - half) + 150, mm2(g, row, half, zj)))

            ns = 0
            for k in range(RR // 2):
                ng = 0
                for op in "0v svv avv 1v svv bvv svv" + (" s" if k == 2 else ""):
                    if op in "01":
                        hidden(zbs[k].at[0, int(op)])
                    elif op in "ab":
                        output(gt16.at[0], xrow(2 * k + "ab".index(op)))
                    elif op == "s":
                        output(kept16.at[SR * i + ns], xs.at[cur, ns])
                        ns += 1
                    elif op == "v":
                        v = conv_ln(ng, [xrow(r) for r in range(2 * k + 3, 2 * k + 7)],
                                    jnp.minimum(RR // 2 * i + k + 2, NR), zbs[(k + 2) % 3], zero)
                        late.append((now[0] + 500, lambda v=v: v))
                        ng += 1
            now[0] += 1000
            advance(0)
            return nxt

        lax.fori_loop(0, NI, body, 0)
        s_out(NI - 1, (NI - 1) % 3).start()
        r_out(NI - 1).start()
        for i in (NI - 2, NI - 1):
            s_out(i, i % 3).wait()
            r_out(i).wait()

    pl.run_scoped(
        pass2,
        pltpu.VMEM((3, SR, C, W), BF16),
        pltpu.VMEM((4 * RR + 1, C, W), BF16),
        pltpu.VMEM((1, TB, 128), F32),
        pltpu.VMEM((1, C, 128), F32),
        [pltpu.VMEM((1, 2, C, W), BF16)] * 3,
        pltpu.VMEM((1, E // 2, W), U32),
    )


@jax.jit
def pallas_standalone__modern_conv_block_convnext_v2__vision_kernel(
    x: jax.Array,
    dw: jax.Array,
    w1: jax.Array,
    w2: jax.Array,
    grn_gamma: jax.Array,
    grn_beta: jax.Array,
):
    tiles = x.reshape(H, NT, 128, NG, 8).transpose(0, 3, 1, 4, 2).reshape(NP, 2, NG * NT, 8, 128)
    rows = x.reshape(H, W, C).transpose(0, 2, 1)
    vmem = pl.BlockSpec(memory_space=pltpu.VMEM)
    hbm = pl.BlockSpec(memory_space=pl.ANY)
    out = pl.pallas_call(
        _kernel,
        out_shape=jax.ShapeDtypeStruct(rows.shape, rows.dtype),
        in_specs=[hbm, hbm, vmem, vmem, vmem, vmem, vmem],
        out_specs=hbm,
        scratch_shapes=[
            pltpu.VMEM((SR * NI, E // 2, W), U32),
            pltpu.VMEM((NR + 1, 8, 128), F32),
            pltpu.VMEM((1, WB, 128), U32),
            pltpu.SMEM((NT,), jnp.int32),
            pltpu.SemaphoreType.DMA((14,)),
        ],
        compiler_params=pltpu.CompilerParams(vmem_limit_bytes=128 << 20, disable_bounds_checks=True),
        name="cnx",
    )(tiles, rows, dw, w1, w2.T, grn_gamma, grn_beta)
    return out.transpose(0, 2, 1).reshape(x.shape)
```

```python
import math

import jax
import jax.numpy as jnp
from jax import lax
import jax.experimental.pallas as pl
import jax.experimental.pallas.tpu as pltpu

F32, BF16, U32 = jnp.float32, jnp.bfloat16, jnp.uint32
H, W, C, E = 512, 512, 96, 384
NG, NT = C // 8, W // 128
NP = H // 2
MC = 64
NM = E // MC

_C0 = math.sqrt(2.0 / math.pi)
_K = (_C0 * 0.044715) ** (1.0 / 3.0)
_B = _C0 / _K
_GS = 0.5 / _K

U = 8
SUMS, SCALE = (0, 1, 2, 3, 4, 5, 6, 7), (4, 5, 6, 7, 8, 9, 10, 11)
NB = NP // U
XN = U + 2
SR, RR = 10, 6
SL = 2
NI = H // (SR + RR)
NR = RR * NI // 2

W1, S1, S2, AN, AW, AC = 0, 192, 264, 336, 352, 448
W2, WB = AW, AC + E
CR, CP, CB = 8 * C, 8 * C + 8, 8 * C + 32
TP, TR, TB = 9 * C, 9 * C + 32, 9 * C + 96


def _tree(v):
    while len(v) > 1:
        v = [v[i] + v[i + 1] if i + 1 < len(v) else v[i] for i in range(0, len(v), 2)]
    return v[0]


def _shift(prv, nxt):
    lane = lax.broadcasted_iota(jnp.int32, (8, 128), 1)
    zero = jnp.zeros_like(prv[0])
    r = [zero] + [pltpu.roll(t, 1, 1) for t in prv]
    l = [pltpu.roll(t, 127, 1) for t in nxt] + [zero]
    return ([jnp.where(lane == 0, r[j], r[j + 1]) for j in range(NT)],
            [jnp.where(lane == 127, l[j + 1], l[j]) for j in range(NT)])


def _gelu(z):
    return z + z * jnp.tanh(z * (z * z + _B))


def _kernel(xt_hbm, x_hbm, dw_ref, w1_ref, w2t_ref, gam_ref, bet_ref, o_hbm, kept, rstd, wb, zs, sem):
    x32 = xt_hbm.bitcast(U32)
    kept16 = kept.bitcast(BF16)
    for j in range(NT):
        zs[j] = 0

    def taps():
        d = dw_ref[...].astype(F32)
        m = jnp.concatenate([d[i, j:j + 1, :] for i in range(3) for j in range(3)] + [jnp.zeros((128 - 9, C), F32)], axis=0)
        m = jnp.concatenate([m, jnp.zeros((128, 128 - C), F32)], axis=1).T[:C]
        return [jnp.broadcast_to(m[:, t:t + 1], (C, 128)) for t in range(9)]

    def mm1(m, n, z):
        lhs = pltpu.bitcast(wb[0, W1 + m * MC // 2:W1 + (m + n) * MC // 2], BF16)[:, :C]
        return jnp.dot(lhs, z, preferred_element_type=F32)

    def put_act(dst, row, m, g):
        dst[pl.ds(row, 1), m * MC:(m + 1) * MC, :] = g[None].astype(BF16)

    def anchor(v, zero):
        wb[zero, AN:AN + 8] = pltpu.bitcast(v[-8:, -128:], U32)

    def pass1(xb, sbs, cbs, zb, raw):
        z16 = zb.bitcast(BF16)

        def load(slot, p_hi, n_hi, off_hi, p_lo, n_lo):
            return [
                pltpu.make_async_copy(x32.at[pl.ds(p_hi - 1, n_hi), 1],
                                      xb.at[slot, pl.ds(off_hi, n_hi), pl.ds(0, 48), pl.ds(0, 4)], sem.at[slot]),
                pltpu.make_async_copy(x32.at[pl.ds(p_lo, n_lo), 0],
                                      xb.at[slot, pl.ds(0, n_lo), pl.ds(0, 48), pl.ds(4, 4)], sem.at[2 + slot]),
            ]

        def block(b, slot):
            return load(slot, b * U + 3, XN, 0, b * U + 3, XN)

        def last_block():
            return load((NB - 1) & 1, NP - U + 3, U - 2, 0, NP - U + 3, U - 3)

        def prep_weights():
            tp = taps()
            r = lax.broadcasted_iota(jnp.int32, (C, 128), 0)
            k = lax.broadcasted_iota(jnp.int32, (C, 128), 1)
            key = jnp.where((r & 7) == (k & 7), k >> 3, -1)
            mats = []
            for o in range(2):
                a = jnp.zeros((C, 128), F32)
                for i in range(3):
                    for j in range(3):
                        a = jnp.where(key == ((i + o) // 2 * 3 + j) * 2 + (i + o) % 2, tp[3 * i + j], a)
                mats.append(a)
            for g in range(NG):
                a = jnp.concatenate([t[8 * g:8 * g + 8] for t in mats], axis=0)
                wb[0, AW + 8 * g:AW + 8 * g + 8] = pltpu.bitcast(a.astype(BF16), U32)
            w = w1_ref[...].astype(F32)
            w = w - jnp.sum(w, axis=0, keepdims=True) * (1.0 / C)
            w = jnp.concatenate([w, jnp.zeros((128 - C, E), F32)], axis=0)
            wb[0, W1:W1 + E // 2] = pltpu.bitcast(w.T.astype(BF16), U32)
            wb[0, AC:AC + E] = jnp.zeros((E, 128), U32)
            raw[...] = jnp.zeros_like(raw)

        def shift(src, g, dst, zero):
            v = [src[NT * g + j] for j in range(NT)]
            for d, part in enumerate(_shift(v, v)):
                for j in range(NT):
                    dst[zero, d, j] = part[j]

        def conv(g, halves, cb, zero):
            cols = [jnp.concatenate([t for src, sb in halves for t in (sb[0, 0, j], src[NT * g + j], sb[0, 1, j])], axis=0)
                    for j in range(NT)]
            res = jnp.dot(pltpu.bitcast(wb[0, AW + 8 * g:AW + 8 * g + 8], BF16)[:, :C],
                          pltpu.bitcast(jnp.concatenate(cols, axis=1), BF16), preferred_element_type=F32)
            for q in range(2 * NT):
                o, j = divmod(q, NT)
                cb[zero, q * C + 8 * g:q * C + 8 * g + 8] = res[8 * o:8 * o + 8, 128 * j:128 * j + 128]

        def ln_sums(q, cb, zero):
            c = [cb[0, q * C + 8 * g:q * C + 8 * g + 8] for g in range(NG)]
            s1, s2 = c[0], c[0] * c[0]
            for t in c[1:]:
                s1, s2 = s1 + t, s2 + t * t
            wb[zero, S1 + 9 * q:S1 + 9 * q + 8] = pltpu.bitcast(s1, U32)
            wb[zero, S2 + 9 * q:S2 + 9 * q + 8] = pltpu.bitcast(s2, U32)

        def ln_rstd(cb, pair, zero):
            s1, s2 = (_tree([pltpu.bitcast(wb[0, pl.ds(s + i, 8, stride=9), :], F32) for i in range(8)]) for s in (S1, S2))
            var = jnp.maximum(s2 - s1 * s1 * (1.0 / C), 0.0)
            r = lax.rsqrt(var * (1.0 / (C * _K * _K)) + 1e-5 / (_K * _K))
            cb[zero, CR:CR + 8] = r
            if pair is not None:
                rstd[jnp.minimum(pair, NR)] = r
            return r

        def ln_scale(q, cb, zrow):
            o, j = divmod(q, NT)
            z = cb[0, q * C:(q + 1) * C] * cb[0, CR + q:CR + q + 1]
            z16[pl.ds(zrow + o, 1), :, 128 * j:128 * j + 128] = z[None].astype(BF16)

        def act(m, z, row, zero):
            g = _gelu(z)
            if row is not None:
                put_act(kept16, row, m, g)
            sq = g * g
            rows = slice(AC + m * MC, AC + (m + 1) * MC)
            tot = pltpu.bitcast(wb[0, rows], F32) + _tree([sq[:, 128 * j:128 * j + 128] for j in range(NT)])
            wb[zero, rows] = pltpu.bitcast(tot, U32)

        def run(slots, xp, p0, first, keep):
            zero = zs[0]
            hid = {}
            live = (lambda p: p >= 0) if first else (lambda p: True)

            def finish(t):
                p, q = divmod(t, 12)
                row = 2 * jnp.maximum(p0 + p - NR, 0) + q // NM if keep else None
                act(q % NM, raw[...] if t < 0 else hid[t], row, zero)

            for t in slots:
                p, q = divmod(t, 12)
                if t - 2 in hid:
                    pin = hid[t - 2][0:8, 0:128]
                    xb[zero, 0, 48] = pltpu.bitcast(pin, U32)
                    if q in SCALE:
                        cbs[(p + 1) & 3][zero, CP:CP + 8] = pin
                n = t + 53
                if live(n // 12):
                    shift(xp(n // 12), n % 12, sbs[n & 15], zero)
                if not first:
                    hid[t] = mm1(q % NM, 1, z16[2 * (p & 1) + q // NM])
                    if t == slots[-1]:
                        raw[...] = hid[t]
                if live(p + 2):
                    if q in SUMS:
                        ln_sums(SUMS.index(q), cbs[(p + 2) & 3], zero)
                    elif q == SUMS[-1] + 1:
                        r = ln_rstd(cbs[(p + 2) & 3], None if keep else p0 + p + 2, zero)
                    elif q == SUMS[-1] + 2:
                        anchor(r, zero)
                for k in range(2 * NT):
                    if live(p + 1) and q == SCALE[k]:
                        ln_scale(k, cbs[(p + 1) & 3], 2 * ((p + 1) & 1) + zero)
                n = t + 38
                if live(n // 12):
                    conv(n % 12, [(xp(n // 12 + k), sbs[(n + 12 * k) & 15]) for k in range(2)], cbs[(n // 12) & 3], zero)
                if not first:
                    for tf in [-1] if t == 0 else range(max(t - 2, 0), t if t == slots[-1] else t - 1):
                        finish(tf)

        head = load(1, 1, 4, 1, 0, 5)
        for cp in head + block(0, 0):
            cp.start()
        prep_weights()
        for cp in head:
            cp.wait()
        xb[1, 0, 0:48, 0:4, :] = jnp.zeros((48, 4, 128), U32)
        run(range(-53, 0), lambda p: xb.at[1, p], 0, True, False)

        def body_dropped(b, carry):
            slot = b & 1
            for cp in block(b, slot):
                cp.wait()
            for cp in block(b + 1, 1 - slot):
                cp.start()
            run(range(12 * U), lambda p: xb.at[slot, p - 3], b * U, False, False)
            return carry

        def body_kept(b, carry):
            slot = b & 1

            @pl.when(b < NB - 1)
            def _():
                for cp in block(b, slot):
                    cp.wait()

            @pl.when(b < NB - 2)
            def _():
                for cp in block(b + 1, 1 - slot):
                    cp.start()

            @pl.when(b >= NB - 2)
            def _():
                @pl.when(b == NB - 1)
                def _():
                    for cp in last_block():
                        cp.wait()
                    xb[(NB - 1) & 1, U - 3, 0:48, 4:8, :] = jnp.zeros((48, 4, 128), U32)

                @pl.when(b == NB - 2)
                def _():
                    for cp in last_block():
                        cp.start()

            run(range(12 * U), lambda p: xb.at[slot, p - 3], b * U, False, True)
            return carry

        lax.fori_loop(0, NR // U, body_dropped, 0)
        lax.fori_loop(NR // U, NB, body_kept, 0)
        act(NM - 1, raw[...], SR * NI - 1, 0)

    pl.run_scoped(
        pass1,
        pltpu.VMEM((2, XN, 50, 8, 128), U32),
        [pltpu.VMEM((1, 2, NT, 8, 128), U32)] * 16,
        [pltpu.VMEM((1, CB, 128), F32)] * 4,
        pltpu.VMEM((4, C // 2, W), U32),
        pltpu.VMEM((MC, W), F32),
    )

    def pass2(xs, xl, xr, tb, bias, zbs, gt):
        gt16 = gt.bitcast(BF16)

        def s_in(i, slot):
            return pltpu.make_async_copy(x_hbm.at[pl.ds(2 * NR + SR * i, SR - SL)], xs.at[slot], sem.at[4 + slot])

        def s_out(i, slot):
            return pltpu.make_async_copy(xs.at[slot], o_hbm.at[pl.ds(2 * NR + SR * i, SR - SL)], sem.at[7 + slot])

        def l_in(i):
            return pltpu.make_async_copy(x_hbm.at[pl.ds(2 * NR + SR * (i + 1) - SL, SL)], xl.at[i & 3], sem.at[18 + (i & 3)])

        def l_out(i):
            return pltpu.make_async_copy(xl.at[i & 3], o_hbm.at[pl.ds(2 * NR + SR * (i + 1) - SL, SL)], sem.at[22 + (i & 3)])

        def r_in(i):
            return pltpu.make_async_copy(x_hbm.at[pl.ds(RR * i, RR - 1)], xr.at[pl.ds(RR * (i & 3), RR - 1)], sem.at[i & 3])

        def r_in_late(i):
            return pltpu.make_async_copy(x_hbm.at[RR * i + RR - 1], xr.at[RR * (i & 3) + RR - 1], sem.at[14 + (i & 3)])

        def r_out(i):
            return pltpu.make_async_copy(xr.at[pl.ds(RR * (i & 3), RR)], o_hbm.at[pl.ds(RR * i, RR)], sem.at[10 + (i & 3)])

        def prep_weights():
            ss = jnp.sum(pltpu.bitcast(wb[0, AC:AC + E], F32).T, axis=0, keepdims=True)
            gx = jnp.sqrt(ss * (_GS * _GS) + 1e-6)
            nx = gx / (jnp.sum(gx, axis=1, keepdims=True) * (1.0 / E) + 1e-6)
            gamma = gam_ref[...].astype(F32).reshape(1, E)
            beta = bet_ref[...].astype(F32).reshape(1, E)
            w2 = w2t_ref[...].astype(F32)
            w2s = pltpu.bitcast((w2 * ((gamma * nx + 1.0) * _GS)).astype(BF16), U32)
            for k in range(E // 128):
                wb[0, W2 + 48 * k:W2 + 48 * k + 48] = w2s[:, 128 * k:128 * k + 128]
            bias[0] = jnp.broadcast_to(jnp.sum(w2 * beta, axis=1, keepdims=True), (C, 128))
            for t, v in enumerate(taps()):
                tb[0, C * t:C * t + C] = v

        def conv_ln(g, rows, pair, zb, zero, before=None):
            if g == 0:
                for q in range(2 * NT):
                    tb[zero, TR + 8 * q:TR + 8 * q + 8] = jnp.broadcast_to(rstd[pair, q:q + 1], (8, 128))
            w = [tb[0, C * t + 8 * g:C * t + 8 * g + 8] for t in range(9)]
            d = [None if r is None else r[8 * g:8 * g + 8, :].astype(F32) for r in rows]
            mids, outs = [], []
            for o in range(2):
                part = [[_tree([d[o + i][:, 128 * j:128 * j + 128] * w[3 * i + dx] for i in range(3) if d[o + i] is not None])
                         for j in range(NT)] for dx in range(3)]
                c = [m + a + b for m, a, b in zip(part[1], *_shift(part[0], part[2]))]
                z = [c[j] * tb[0, TR + 8 * (NT * o + j):TR + 8 * (NT * o + j) + 8] for j in range(NT)]
                zb[zero, o, 8 * g:8 * g + 8, :] = jnp.concatenate(z, axis=1).astype(BF16)
                mids += part[1]
                outs += c
            done = outs[7] if before is None else _tree(outs)
            pin = done if before is None else _tree(mids + before)
            if before is None:
                for n in range(4):
                    tb[zero, TP + 8 * n:TP + 8 * n + 8] = outs[2 * n] + outs[2 * n + 1]
            else:
                tb[zero, TP:TP + 8] = pin
            xr[4 * RR + zero, 0:8, 0:256] = jnp.concatenate([mids[3], mids[7]] if before is None else [pin, pin], axis=1).astype(BF16)
            return done

        def mm2(g, xrow, half, zj):
            lhs = pltpu.bitcast(jnp.concatenate([wb[0, W2 + 48 * k:W2 + 48 * k + 48] for k in range(E // 128)], axis=1), BF16)
            o = [jnp.dot(lhs, g[:, 128 * j:128 * j + 128], preferred_element_type=F32) + bias[zj[j]]
                 for j in (2 * half, 2 * half + 1)]

            def finish():
                res = jnp.concatenate(o, axis=1) + xrow[:, 256 * half:256 * half + 256].astype(F32)
                xrow[:, 256 * half:256 * half + 256] = res.astype(BF16)
                return res
            return finish

        r_in(0).start()
        r_in(1).start()
        s_in(0, 0).start()
        l_in(0).start()
        r_in_late(0).start()
        r_in_late(1).start()
        l_in(1).start()
        prep_weights()
        r_in(0).wait()
        before = []
        for p in range(2):
            for g in range(NG):
                rows = [None if r < 0 else xr.at[r] for r in range(2 * p - 1, 2 * p + 3)]
                before = [conv_ln(g, rows, p, zbs[p], zs[0], before)]

        def body(i, cur):
            zj = [zs[j] for j in range(NT)]
            zero = zj[0]
            prv = jnp.where(cur == 0, 2, cur - 1)
            nxt = jnp.where(cur == 2, 0, cur + 1)

            @pl.when(i >= 2)
            def _():
                s_out(i - 2, nxt).wait()
                r_out(i - 2).wait()
                l_out(i - 2).wait()

            @pl.when(i < NI - 1)
            def _():
                r_in(i + 2).start()
                s_in(i + 1, nxt).start()
                r_in_late(i + 2).start()

            @pl.when(i < NI - 2)
            def _():
                l_in(i + 2).start()

            @pl.when(i >= 1)
            def _():
                s_out(i - 1, prv).start()
                r_out(i - 1).start()
                l_out(i - 1).start()

            r_in(i + 1).wait()
            s_in(i, cur).wait()
            l_in(i).wait()
            r_in_late(i).wait()

            def xrow(r):
                return xr.at[RR * ((i + r // RR) & 3) + r % RR]

            late = []
            now = [0]

            def advance(cycles):
                for deadline, work in late:
                    if deadline <= now[0]:
                        anchor(work(), zero)
                late[:] = [w for w in late if w[0] > now[0]]
                now[0] += cycles

            def hidden(z):
                advance(E)
                h = mm1(0, NM, z[...])

                def finish(m):
                    g = _gelu(h[m * MC:(m + 1) * MC])
                    put_act(gt16, zero, m, g)
                    return g
                late.extend((now[0] - (NM - 1 - m) * MC + 160, lambda m=m: finish(m)) for m in range(NM))

            def output(g, row):
                for half in range(2):
                    advance(C * (1 + half))
                    late.append((now[0] + C * (1 - half) + 150, mm2(g, row, half, zj)))

            ns = 0
            for k in range(RR // 2):
                ng = 0
                for op in "0v svv avv 1v svv bvv svv" + (" s" if k == 2 else ""):
                    if op in "01":
                        hidden(zbs[k].at[0, int(op)])
                    elif op in "ab":
                        output(gt16.at[0], xrow(2 * k + "ab".index(op)))
                    elif op == "s":
                        output(kept16.at[SR * i + ns], xs.at[cur, ns] if ns < SR - SL else xl.at[i & 3, ns - SR + SL])
                        ns += 1
                    elif op == "v":
                        v = conv_ln(ng, [xrow(r) for r in range(2 * k + 3, 2 * k + 7)],
                                    jnp.minimum(RR // 2 * i + k + 2, NR), zbs[(k + 2) % 3], zero)
                        late.append((now[0] + 500, lambda v=v: v))
                        ng += 1
            now[0] += 1000
            advance(0)
            return nxt

        lax.fori_loop(0, NI, body, 0)
        s_out(NI - 1, (NI - 1) % 3).start()
        r_out(NI - 1).start()
        l_out(NI - 1).start()
        r_in_late(NI).wait()
        for i in (NI - 2, NI - 1):
            s_out(i, i % 3).wait()
            r_out(i).wait()
            l_out(i).wait()

    pl.run_scoped(
        pass2,
        pltpu.VMEM((3, SR - SL, C, W), BF16),
        pltpu.VMEM((4, SL, C, W), BF16),
        pltpu.VMEM((4 * RR + 1, C, W), BF16),
        pltpu.VMEM((1, TB, 128), F32),
        pltpu.VMEM((1, C, 128), F32),
        [pltpu.VMEM((1, 2, C, W), BF16)] * 3,
        pltpu.VMEM((1, E // 2, W), U32),
    )


@jax.jit
def pallas_standalone__modern_conv_block_convnext_v2__vision_kernel(
    x: jax.Array,
    dw: jax.Array,
    w1: jax.Array,
    w2: jax.Array,
    grn_gamma: jax.Array,
    grn_beta: jax.Array,
):
    tiles = x.reshape(H, NT, 128, NG, 8).transpose(0, 3, 1, 4, 2).reshape(NP, 2, NG * NT, 8, 128)
    rows = x.reshape(H, W, C).transpose(0, 2, 1)
    vmem = pl.BlockSpec(memory_space=pltpu.VMEM)
    hbm = pl.BlockSpec(memory_space=pl.ANY)
    out = pl.pallas_call(
        _kernel,
        out_shape=jax.ShapeDtypeStruct(rows.shape, rows.dtype),
        in_specs=[hbm, hbm, vmem, vmem, vmem, vmem, vmem],
        out_specs=hbm,
        scratch_shapes=[
            pltpu.VMEM((SR * NI, E // 2, W), U32),
            pltpu.VMEM((NR + 1, 8, 128), F32),
            pltpu.VMEM((1, WB, 128), U32),
            pltpu.SMEM((NT,), jnp.int32),
            pltpu.SemaphoreType.DMA((26,)),
        ],
        compiler_params=pltpu.CompilerParams(vmem_limit_bytes=128 << 20, disable_bounds_checks=True),
        name="convnext_v2_block",
    )(tiles, rows, dw, w1, w2.T, grn_gamma, grn_beta)
    return out.transpose(0, 2, 1).reshape(x.shape)
```
